```python
import os as _os
_os.environ.setdefault('JAX_PLATFORMS', 'cpu')
import jax
import jax.numpy as jnp

def _softmax(x, axis=-1):
    return jax.nn.softmax(x, axis=axis)

def _gelu(x):
    return jax.nn.gelu(x, approximate=True)

def _silu(x):
    return jax.nn.silu(x)

def _sigmoid(x):
    return jax.nn.sigmoid(x)

def _layernorm(x, axis=-1, eps=1e-05):
    m = jnp.mean(x, axis=axis, keepdims=True)
    v = jnp.var(x, axis=axis, keepdims=True)
    return (x - m) / jnp.sqrt(v + eps)

def _scatter_add(tgt, idx, src, axis=0):
    return tgt.at[idx].add(src)

def _segment_sum(src, seg, n):
    return jax.ops.segment_sum(src, seg, n)

class _Rng:

    def __init__(self, key):
        self._k = key

    def _next(self):
        self._k, sub = jax.random.split(self._k)
        return sub

    def normal(self, shape):
        return jax.random.normal(self._next(), shape, dtype=jnp.bfloat16)

    def randint(self, lo, hi, shape):
        return jax.random.randint(self._next(), shape, lo, hi, dtype=jnp.int32)

    def uniform(self, shape, lo=0.0, hi=1.0):
        return jax.random.uniform(self._next(), shape, jnp.bfloat16, lo, hi)

    def permutation(self, n):
        return jax.random.permutation(self._next(), n)
kernel_name = 'gated_mix__sliding_block__memory_aug_recurrent_mem_tr__prompt'

def setup_inputs():
    _rng = _Rng(jax.random.key(int.from_bytes(__import__("os").urandom(4), "little")))
    _w = lambda a: (lambda t: t.astype(jnp.bfloat16) if jnp.issubdtype(t.dtype, jnp.floating) else t)(jnp.asarray(a))

    def _A_setup():
        B, S, D = (1, 2048, 448)
        return {'x': _w((lambda *s: _rng.normal(s) * 0.05)(B, S, D)), 'wqkv': _w((lambda *s: _rng.normal(s) * 0.8)(D, 3 * D)), 'wo': _w((lambda *s: _rng.normal(s) * 0.05)(D, D))}
    _A_in = _A_setup()

    def _B_setup():
        B, S, Dm = (1, 2048, 448)
        H, Dh = (16, 256)
        M, seg = (8, 32)
        seg = min(seg, S)
        S = S // seg * seg
        return {'x': _w((lambda *s: _rng.normal(s) * 0.05)(B, S, Dm)), 'mem0': _w((lambda *s: _rng.normal(s) * 0.8)(B, M, Dm)), 'Wq': _w((lambda *s: _rng.normal(s) * 3.2)(Dm, H, Dh) * Dm ** (-0.5)), 'Wk': _w((lambda *s: _rng.normal(s) * 3.2)(Dm, H, Dh) * Dm ** (-0.5)), 'Wv': _w((lambda *s: _rng.normal(s) * 0.8)(Dm, H, Dh) * Dm ** (-0.5)), 'Wo': _w((lambda *s: _rng.normal(s) * 0.8)(H, Dh, Dm) * (H * Dh) ** (-0.5)), 'seg_len': seg}
    _B_in = _B_setup()
    return {'A_x': _A_in['x'], 'A_wqkv': _A_in['wqkv'], 'A_wo': _A_in['wo'], 'B_x': _B_in['x'], 'B_mem0': _B_in['mem0'], 'B_Wq': _B_in['Wq'], 'B_Wk': _B_in['Wk'], 'B_Wv': _B_in['Wv'], 'B_Wo': _B_in['Wo'], 'B_seg_len': _B_in['seg_len'], 'gate_w': _w((lambda *s: _rng.normal(s) * 0.05)(448) * 16.0)}

def reference(A_x, A_wqkv, A_wo, B_x, B_mem0, B_Wq, B_Wk, B_Wv, B_Wo, B_seg_len, gate_w):

    def _A_ref(x, wqkv, wo):
        B, S, D = x.shape
        H = 16
        Dh = D // H
        W = 256
        qkv = (lambda x, *d: x.transpose(*d))((x @ wqkv).reshape(B, S, 3, H, Dh), 2, 0, 3, 1, 4)
        q, k, v = (qkv[0], qkv[1], qkv[2])
        scores = jnp.einsum('bhqd,bhkd->bhqk', q, k) * Dh ** (-0.5)
        idx = jnp.arange(S)
        mask = (idx[:, None] - idx[None, :] >= 0) & (idx[:, None] - idx[None, :] < W)
        scores = jnp.where(mask[None, None], scores, -1000000000.0)
        p = _softmax(scores, axis=-1)
        o = jnp.einsum('bhqk,bhkd->bhqd', p, v)
        return (lambda x, *d: x.transpose(*d))(o, 0, 2, 1, 3).reshape(B, S, D) @ wo

    def _B_ref(x, mem0, Wq, Wk, Wv, Wo, seg_len):
        B, S, Dm = x.shape
        H, Dh = (Wq.shape[1], Wq.shape[2])
        M = mem0.shape[1]
        scale = Dh ** (-0.5)
        n_seg = S // seg_len
        L = M + seg_len
        idx = jnp.arange(L)
        mask = (idx[:, None] < M) | (idx[:, None] >= idx[None, :])
        mem = mem0
        outs = []
        for s in range(n_seg):
            xs = x[:, s * seg_len:(s + 1) * seg_len, :].copy()
            h = jnp.concatenate([mem, xs], axis=1)
            q = jnp.einsum('btd,dhe->bhte', h, Wq)
            k = jnp.einsum('btd,dhe->bhte', h, Wk)
            v = jnp.einsum('btd,dhe->bhte', h, Wv)
            scores = jnp.einsum('bhqe,bhke->bhqk', q, k) * scale
            scores = jnp.where(mask[None, None], scores, -1000000000.0)
            p = _softmax(scores, axis=-1)
            o = jnp.einsum('bhqk,bhke->bhqe', p, v)
            o = jnp.einsum('bhte,hed->btd', o, Wo)
            mem = o[:, :M, :].copy()
            outs.append(o[:, M:, :])
        return jnp.concatenate(outs, axis=1)
    x = A_x
    g = _sigmoid((x * gate_w).sum(-1, keepdims=True))
    a = _A_ref(x, A_wqkv, A_wo)
    b = _B_ref(x, B_mem0, B_Wq, B_Wk, B_Wv, B_Wo, B_seg_len)
    return g * a + (1 - g) * b
```

```python
import functools
import math

import jax
import jax.numpy as jnp
from jax import lax
from jax.experimental import pallas as pl
from jax.experimental.pallas import tpu as pltpu

F32 = jnp.float32
BF16 = jnp.bfloat16
U32 = jnp.uint32
LOG2E = math.log2(math.e)
NEG = -1e9

NT = (((1,), (1,)), ((), ()))

DO_A = True
DO_B = True


def _dot(a, b):
    return jnp.dot(a, b, preferred_element_type=F32)


def _dot_nt(a, b):
    return lax.dot_general(a, b, NT, preferred_element_type=F32)


def _bf16_round(v):
    import numpy as np
    import ml_dtypes
    return float(np.asarray(v, dtype=ml_dtypes.bfloat16).astype(np.float32))


def _make_kernel(S, D, HA, W, HB, E, M, SEG):
    DHA = D // HA
    SLOT = 32
    DP = HA * SLOT
    QB = 128
    NQB = S // QB
    NPAIR = S // (2 * SEG)
    HE = HB * E
    assert SEG == 32 and M == 8 and W == 2 * QB and D % 16 == 0
    GPH = 128 // SLOT
    NG = HA // GPH
    GW = GPH * DHA
    cexp_a = _bf16_round(DHA ** -0.5) * LOG2E
    cexp_b = _bf16_round(E ** -0.5) * LOG2E
    PCH = 256

    def kernel(xaT_hbm, wqkv_hbm, wo_hbm, mem0_ref, wq_hbm, wk_hbm, wv_hbm, woT_hbm, gate_ref,
               outT_hbm,
               xaT, wqkv, wo, xb, wraw, wpk, woTraw, wob, wTp, woTp, qT, kk, vT, gl, gaT, bb, outT, sems):
        cps = {}

        def start(name, src, dst, idx):
            cp = pltpu.make_async_copy(src, dst, sems.at[idx])
            cp.start()
            cps[name] = cp
        start("wqkv", wqkv_hbm, wqkv, 1)
        start("xa", xaT_hbm, xaT, 0)
        start("wo", wo_hbm, wo, 2)
        start("wob", woT_hbm, woTraw, 10)
        for mi, w_hbm in enumerate((wq_hbm, wk_hbm, wv_hbm)):
            wu = w_hbm.bitcast(U32)
            for t in range(2):
                start(f"w{mi}{t}", wu.at[:, t * 128:(t + 1) * 128], wraw.at[mi, t], 4 + 2 * mi + t)

        cps["wqkv"].wait()
        r_i = lax.broadcasted_iota(jnp.int32, (128, GW), 0)
        c_i = lax.broadcasted_iota(jnp.int32, (128, GW), 1)
        selT = ((r_i // SLOT == c_i // DHA) & (r_i % SLOT == c_i % DHA)).astype(BF16)
        wqkvT = wqkv[...].T
        for r in range(3 * NG):
            wTp[r * 128:(r + 1) * 128, :] = _dot(selT, wqkvT[r * GW:(r + 1) * GW, :]).astype(BF16)
        wTp[3 * DP:3 * DP + 16, :] = jnp.broadcast_to(gate_ref[...], (16, D))
        cps["wo"].wait()
        wo_v = wo[...]
        wo_pad = jnp.concatenate([_dot(selT, wo_v[r * GW:(r + 1) * GW, :]) for r in range(NG)], axis=0)
        woTp[...] = wo_pad.T.astype(BF16)
        kk[0:W, :] = jnp.zeros((W, DP), BF16)
        vT[:, 0:W] = jnp.zeros((DP, W), BF16)

        cps["xa"].wait()

        def proj(c, carry):
            col = pl.multiple_of(c * PCH, PCH)
            xc = xaT[:, pl.ds(col, PCH)]
            qT[:, pl.ds(col, PCH)] = _dot(wTp[0:DP, :], xc).astype(BF16)
            kk[pl.ds(W + col, PCH), :] = _dot(wTp[DP:2 * DP, :], xc).astype(BF16).T
            r = _dot(wTp[2 * DP:3 * DP + 16, :], xc)
            vT[:, pl.ds(W + col, PCH)] = r[0:DP].astype(BF16)
            gl[:, pl.ds(col, PCH)] = jax.nn.sigmoid(r[DP:DP + 8])
            return carry
        if DO_A:
            lax.fori_loop(0, S // PCH, proj, 0)

        krow = lax.broadcasted_iota(jnp.int32, (QB, QB), 0)
        qcol = lax.broadcasted_iota(jnp.int32, (QB, QB), 1)
        upper = krow > qcol
        hrow = lax.broadcasted_iota(jnp.int32, (128, QB), 0) // SLOT

        def attn_block(i, nblk):
            q0 = pl.multiple_of(i * QB, QB)
            k0 = pl.multiple_of(i * QB + (3 - nblk) * QB, QB)
            nk = nblk * QB
            oTs = []

            def scores(g):
                kg = kk[pl.ds(k0, nk), g * 128:(g + 1) * 128]
                qg = qT[g * 128:(g + 1) * 128, pl.ds(q0, QB)]
                wq4 = jnp.concatenate([jnp.where(hrow == j, qg, jnp.zeros_like(qg)) for j in range(GPH)], axis=1)
                return _dot(kg, wq4)

            def finish(g, s4):
                for j in range(GPH):
                    h = g * GPH + j
                    s = s4[:, j * QB:(j + 1) * QB]
                    s2 = s[(nblk - 1) * QB:nblk * QB]
                    if nblk == 3:
                        c = jnp.where(upper, s[0:QB], s2)
                    else:
                        c = jnp.where(upper, NEG, s2)
                    m = jnp.max(c, axis=0, keepdims=True)
                    if nblk >= 2:
                        s1 = s[(nblk - 2) * QB:(nblk - 1) * QB]
                        m = jnp.maximum(m, jnp.max(s1, axis=0, keepdims=True))
                    pc = jnp.exp2((c - m) * cexp_a)
                    l = jnp.sum(pc, axis=0, keepdims=True)
                    parts = []
                    if nblk == 3:
                        parts.append(jnp.where(upper, pc, 0.0).astype(BF16))
                    if nblk >= 2:
                        p1 = jnp.exp2((s1 - m) * cexp_a)
                        l = l + jnp.sum(p1, axis=0, keepdims=True)
                        parts.append(p1.astype(BF16))
                    parts.append(jnp.where(upper, 0.0, pc).astype(BF16))
                    p = jnp.concatenate(parts, axis=0)
                    vh = vT[h * SLOT:(h + 1) * SLOT, pl.ds(k0, nk)]
                    o = _dot(vh, p)
                    oTs.append((o * (1.0 / l)).astype(BF16))

            s_prev = scores(0)
            for g in range(1, NG):
                s_next = scores(g)
                finish(g - 1, s_prev)
                s_prev = s_next
            finish(NG - 1, s_prev)
            oT = jnp.concatenate(oTs, axis=0)
            aT = _dot(woTp[...], oT)
            aT = aT.astype(BF16).astype(F32)
            gaT[:, pl.ds(q0, QB)] = aT * gl[0:1, pl.ds(q0, QB)]

        if DO_A:
            attn_block(0, 1)
            attn_block(1, 2)

            def attn_loop(i, carry):
                attn_block(i, 3)
                return carry
            lax.fori_loop(2, NQB, attn_loop, 0)
        else:
            gaT[...] = jnp.zeros_like(gaT)
            gl[...] = jnp.zeros_like(gl)

        for c in range(S // 256):
            xb[c * 256:(c + 1) * 256, :] = xaT[:, c * 256:(c + 1) * 256].T
        cps["wob"].wait()
        for h in range(HB):
            wob[h * E:(h + 1) * E, :] = woTraw[h * D:(h + 1) * D, :].T
        for mi in range(3):
            for t in range(2):
                cps[f"w{mi}{t}"].wait()
                for j in range(HB // 2):
                    xe = wraw[mi, t, pl.ds(j, D // 2, stride=HB), :]
                    xo = wraw[mi, t, pl.ds(HB // 2 + j, D // 2, stride=HB), :]
                    lo = (xe & U32(0xFFFF)) | (xo << 16)
                    hi = (xe >> 16) | (xo & U32(0xFFFF0000))
                    c0 = (2 * j) * 3 * E + mi * E + t * 128
                    c1 = (2 * j + 1) * 3 * E + mi * E + t * 128
                    wpk[:, c0:c0 + 128] = lo
                    wpk[:, c1:c1 + 128] = hi

        L = 48
        row = lax.broadcasted_iota(jnp.int32, (L, L), 0)
        col = lax.broadcasted_iota(jnp.int32, (L, L), 1)
        validA = (col < M) | ((col < M + SEG) & ((col <= row) | (row < M)))
        capA = jnp.where(validA, jnp.inf, NEG).astype(F32)

        def tok(p):
            return jnp.where(p < 32, p + 32, p - 8)
        validB = (col < M) | ((tok(col) >= SEG) & ((tok(col) <= tok(row)) | (row < M)))
        capB = jnp.where(validB, jnp.inf, NEG).astype(F32)

        def softmax_p(s, cap):
            s = jnp.minimum(s, cap)
            m = jnp.max(s, axis=-1, keepdims=True)
            e = jnp.exp2((s - m) * cexp_b)
            l = jnp.sum(e, axis=-1, keepdims=True)
            return (e * (1.0 / l)).astype(BF16)

        def seg_step(hin, extra, cap, o_post):
            qkv = [None] * HB
            p = [None] * HB
            o = [None] * HB
            tails = [None] * HB

            def do_qkv(h):
                w = pltpu.bitcast(wpk[:, h * 3 * E:(h + 1) * 3 * E], BF16)
                r = _dot(hin, w).astype(BF16)
                if extra is not None:
                    r = jnp.concatenate([r, extra[h]], axis=0)
                else:
                    tails[h] = r[32:48]
                qkv[h] = r

            def do_s(h):
                p[h] = softmax_p(_dot_nt(qkv[h][:, :E], qkv[h][:, E:2 * E]), cap)

            def do_pv(h):
                o[h] = o_post(h, _dot(p[h], qkv[h][:, 2 * E:]))

            for t in range(HB):
                do_qkv(t)
                if t >= 1:
                    do_s(t - 1)
                if t >= 2:
                    do_pv(t - 2)
            acc = None

            def do_wo(h, acc):
                r = _dot(o[h], wob[h * E:(h + 1) * E, :])
                return r if acc is None else acc + r
            for h in range(0, 4):
                acc = do_wo(h, acc)
            do_s(HB - 1)
            do_pv(HB - 2)
            for h in range(4, 9):
                acc = do_wo(h, acc)
            do_pv(HB - 1)
            for h in range(9, HB):
                acc = do_wo(h, acc)
            return acc, tails

        def pair(i, mem):
            base = pl.multiple_of(i * 64, 64)
            t8 = xb[pl.ds(base, 8), :].astype(F32)
            g0 = jnp.concatenate([mem, t8], axis=0).astype(BF16)
            g12 = xb[pl.ds(base + 8, 32), :]
            hA = jnp.concatenate([g0, g12], axis=0)
            saved = [None] * HB

            def postA(h, oh):
                saved[h] = oh[32:40]
                return oh[0:32].astype(BF16)
            resA, tails = seg_step(hA, None, capA, postA)
            mem1 = resA[0:8].astype(BF16).astype(F32)
            t8b = xb[pl.ds(base + 40, 8), :].astype(F32)
            g0b = jnp.concatenate([mem1, t8b], axis=0).astype(BF16)
            g1b = xb[pl.ds(base + 48, 16), :]
            hB = jnp.concatenate([g0b, g1b], axis=0)

            def postB(h, oh):
                return jnp.concatenate([oh[0:32], saved[h], oh[40:48]], axis=0).astype(BF16)
            resB, _ = seg_step(hB, tails, capB, postB)
            mem2 = resB[0:8].astype(BF16).astype(F32)
            b64 = jnp.concatenate([resA[8:32], resB[32:48], resB[8:32]], axis=0)
            bb[pl.ds(base, 64), :] = b64.astype(BF16)
            return mem2

        if DO_B:
            lax.fori_loop(0, NPAIR, pair, mem0_ref[...].astype(F32))
        else:
            bb[...] = jnp.zeros_like(bb)

        ocps = []
        for c in range(NQB):
            sl = slice(c * QB, (c + 1) * QB)
            bT = bb[sl, :].T.astype(F32)
            g = gl[0:1, sl]
            outT[:, sl] = (gaT[:, sl] + (1.0 - g) * bT).astype(BF16)
            cp = pltpu.make_async_copy(outT.at[:, sl], outT_hbm.at[:, sl], sems.at[12 + c])
            cp.start()
            ocps.append(cp)
        for cp in ocps:
            cp.wait()

    return kernel


@functools.partial(jax.jit, static_argnames=("B_seg_len",))
def pallas_gated_mix__sliding_block__memory_aug_recurrent_mem_tr__prompt_kernel(A_x, A_wqkv, A_wo, B_x, B_mem0, B_Wq, B_Wk, B_Wv, B_Wo, B_seg_len, gate_w):
    Bn, S, D = A_x.shape
    assert Bn == 1
    HB, E = B_Wq.shape[1], B_Wq.shape[2]
    M = B_mem0.shape[1]
    HA, WIN = 16, 256
    kern = _make_kernel(S, D, HA, WIN, HB, E, M, B_seg_len)
    hbm_spec = pl.BlockSpec(memory_space=pltpu.MemorySpace.HBM)
    vmem_spec = pl.BlockSpec(memory_space=pltpu.VMEM)
    outT = pl.pallas_call(
        kern,
        out_shape=jax.ShapeDtypeStruct((D, S), BF16),
        in_specs=[hbm_spec, hbm_spec, hbm_spec, vmem_spec, hbm_spec, hbm_spec, hbm_spec, hbm_spec, vmem_spec],
        out_specs=hbm_spec,
        scratch_shapes=[
            pltpu.VMEM((D, S), BF16),
            pltpu.VMEM((D, 3 * D), BF16),
            pltpu.VMEM((D, D), BF16),
            pltpu.VMEM((S, D), BF16),
            pltpu.VMEM((3, 2, D * HB // 2, 128), U32),
            pltpu.VMEM((D // 2, 3 * HB * E), U32),
            pltpu.VMEM((HB * D, E), BF16),
            pltpu.VMEM((HB * E, D), BF16),
            pltpu.VMEM((3 * 512 + 16, D), BF16),
            pltpu.VMEM((D, 512), BF16),
            pltpu.VMEM((512, S), BF16),
            pltpu.VMEM((WIN + S, 512), BF16),
            pltpu.VMEM((512, WIN + S), BF16),
            pltpu.VMEM((8, S), F32),
            pltpu.VMEM((D, S), F32),
            pltpu.VMEM((S, D), BF16),
            pltpu.VMEM((D, S), BF16),
            pltpu.SemaphoreType.DMA((12 + S // 128,)),
        ],
        compiler_params=pltpu.CompilerParams(vmem_limit_bytes=110 * 1024 * 1024),
    )(A_x.reshape(S, D).T, A_wqkv, A_wo, B_mem0.reshape(M, D),
      B_Wq.reshape(D * HB, E), B_Wk.reshape(D * HB, E), B_Wv.reshape(D * HB, E),
      jnp.transpose(B_Wo, (0, 2, 1)).reshape(HB * D, E), gate_w.reshape(1, D))
    return outT.T.reshape(1, S, D)
```

```python
import functools
import math

import jax
import jax.numpy as jnp
from jax import lax
from jax.experimental import pallas as pl
from jax.experimental.pallas import tpu as pltpu

F32 = jnp.float32
BF16 = jnp.bfloat16
U32 = jnp.uint32
LOG2E = math.log2(math.e)
NEG = -1e9

NT = (((1,), (1,)), ((), ()))

DMA_ORDER = (("w", 0, 0), ("wo", 0), ("w", 0, 1), ("w", 1, 0), ("wo", 1), ("w", 1, 1), ("wo", 2), ("wo", 3),
             ("w", 2, 0), ("w", 2, 1))
FIN_T = (5, 7, 9, 11)
S_POS = ('end', 'end')
COMB_T = 2
QFIRST = 0
NS_POS = 'end'
SPLIT_S = 0
S2_T = 5
AOUT_T = 14
LAG_E = (1, 3, 3)
LAG_O = (2, 4, 2)


def _dot(a, b):
    return jnp.dot(a, b, preferred_element_type=F32)


def _dot_nt(a, b):
    return lax.dot_general(a, b, NT, preferred_element_type=F32)


def _bf16_round(v):
    m, e = math.frexp(v)
    return math.ldexp(round(m * 256.0) / 256.0, e)


def _make_kernel(S, D, HA, W, HB, E, M, SEG):
    DHA = D // HA
    SLOT = 32
    DP = HA * SLOT
    QB = 128
    NQB = S // QB
    HE = HB * E
    assert SEG == 32 and M == 8 and W == 2 * QB and D % 16 == 0 and DHA < SLOT
    GPH = 128 // SLOT
    NG = HA // GPH
    GW = GPH * DHA
    cexp_a = _bf16_round(DHA ** -0.5) * LOG2E
    cexp_b = _bf16_round(E ** -0.5) * LOG2E
    PCH = 256

    def kernel(xaT_hbm, wqkv_hbm, wo_hbm, mem0_hbm, wq_hbm, wk_hbm, wv_hbm, woT_hbm, gate_hbm,
               outT_hbm,
               xaT, wqkv, wo, xb, wraw, wpk, woTraw, wob, wTp, woTp, qT, kk, vT, gl, gaT, bb, outT, s0buf, mem0_ref, gate_ref, sems):
        cps = {}

        def start(name, src, dst, idx):
            cp = pltpu.make_async_copy(src, dst, sems.at[idx])
            cp.start()
            cps[name] = cp
        start("wqkv", wqkv_hbm, wqkv, 0)
        start("gate", gate_hbm, gate_ref, 32)
        start("mem0", mem0_hbm, mem0_ref, 33)
        start("xa", xaT_hbm, xaT, 1)
        start("wo", wo_hbm, wo, 2)

        def w_copy(mi, t, par):
            wu = (wq_hbm, wk_hbm, wv_hbm)[mi].bitcast(U32)
            dst = wraw.at[(mi * 2 + t) * 2 + par].reshape(D // 2, HB // 2, 128)
            return pltpu.make_async_copy(wu.at[:, par * (HB // 2):(par + 1) * (HB // 2), t * 128:(t + 1) * 128],
                                         dst, sems.at[4 + (mi * 2 + t) * 2 + par])
        def w_wait(mi, t):
            for par in range(2):
                w_copy(mi, t, par).wait()

        NWO = 4
        HPW = HB // NWO

        def wo_copy(k):
            r0 = pl.multiple_of(k * HPW * D, 16)
            return pltpu.make_async_copy(woT_hbm.at[pl.ds(r0, HPW * D)], woTraw.at[pl.ds(r0, HPW * D)], sems.at[34 + k])

        for item in DMA_ORDER:
            if item[0] == "w":
                for par in range(2):
                    w_copy(item[1], item[2], par).start()
            else:
                wo_copy(item[1]).start()

        cps["wqkv"].wait()
        def respace(r, fill):
            n = r.shape[1]
            first = lax.broadcasted_iota(jnp.int32, (SLOT - DHA, n), 0) == 0
            pad = jnp.where(first, fill, 0.0).astype(r.dtype)
            parts = []
            for h in range(HA):
                parts += [r[h * DHA:(h + 1) * DHA], pad]
            return jnp.concatenate(parts, axis=0)

        wTp[0:3 * D, :] = wqkv[...].T
        cps["gate"].wait()
        cps["mem0"].wait()
        wTp[3 * D:3 * D + 16, :] = jnp.broadcast_to(gate_ref[...].reshape(1, D), (16, D))
        cps["wo"].wait()
        woTp[...] = respace(wo[...].astype(F32), 0.0).T.astype(BF16)
        lane = lax.broadcasted_iota(jnp.int32, (W, DP), 1)
        kk[0:W, :] = jnp.where(lane % SLOT == DHA, NEG, 0.0).astype(BF16)
        vT[:, 0:W] = jnp.zeros((DP, W), BF16)
        gaT[:, 0:QB] = jnp.zeros((D, QB), F32)
        bb[0:QB, :] = jnp.zeros((QB, D), BF16)

        cps["xa"].wait()

        def proj(c):
            col = pl.multiple_of(c * PCH, PCH)
            xc = xaT[:, pl.ds(col, PCH)]
            qT[:, pl.ds(col, PCH)] = respace(_dot(wTp[0:D, :], xc) * cexp_a, 1.0).astype(BF16)
            kk[pl.ds(W + col, PCH), :] = respace(_dot(wTp[D:2 * D, :], xc), 0.0).astype(BF16).T
            r = _dot(wTp[2 * D:3 * D + 16, :], xc)
            vT[:, pl.ds(W + col, PCH)] = respace(r[0:D], 1.0).astype(BF16)
            gl[:, pl.ds(col, PCH)] = jax.nn.sigmoid(r[D:D + 8])

        def xb_chunk(k):
            col = pl.multiple_of(k * 256, 256)
            xb[pl.ds(col, 256), :] = xaT[:, pl.ds(col, 256)].T

        def wob_head(h):
            wob[pl.ds(pl.multiple_of(h * E, E), E), :] = woTraw[pl.ds(pl.multiple_of(h * D, 16), D), :].T

        def w_unit(u):
            mt = u // (HB // 2)
            j = u % (HB // 2)
            mi = mt // 2
            t = mt % 2
            xe = wraw[2 * mt, pl.ds(j, D // 2, stride=HB // 2), :]
            xo = wraw[2 * mt + 1, pl.ds(j, D // 2, stride=HB // 2), :]
            lo = (xe & U32(0xFFFF)) | (xo << 16)
            hi = (xe >> 16) | (xo & U32(0xFFFF0000))
            c0 = pl.multiple_of((2 * j) * 3 * E + mi * E + t * 128, 128)
            wpk[:, pl.ds(c0, 128)] = lo
            wpk[:, pl.ds(c0 + 3 * E, 128)] = hi

        NPC = S // PCH
        assert NPC == 8

        NP1 = 3

        def p1(c, carry):
            proj(c)
            xb_chunk(c)
            return carry
        lax.fori_loop(0, NP1, p1, 0)

        def p3(c, carry):
            for n in range(NPC - NP1):
                @pl.when(c == NP1 + n)
                def _():
                    w_wait(n // 2, n % 2)
                    if n == 0:
                        wo_copy(0).wait()
                    elif n >= 2:
                        wo_copy(n - 1).wait()
            proj(c)
            xb_chunk(c)
            for k in range(HB // 2):
                w_unit((c - NP1) * (HB // 2) + k)
            piece = jnp.maximum(c - NP1 - 1, 0)
            for n in range(HPW):
                wob_head(piece * HPW + n)
            return carry
        lax.fori_loop(NP1, NPC, p3, 0)
        w_wait(2, 1)

        def p4(u, carry):
            w_unit(5 * (HB // 2) + 2 * u)
            w_unit(5 * (HB // 2) + 2 * u + 1)
            return carry
        lax.fori_loop(0, HB // 4, p4, 0)

        krow = lax.broadcasted_iota(jnp.int32, (QB, QB), 0)
        qcol = lax.broadcasted_iota(jnp.int32, (QB, QB), 1)
        upper = krow > qcol

        def a_scores(q0, g, js):
            kg = kk[pl.ds(q0, 3 * QB), g * 128:(g + 1) * 128]
            qg = qT[g * 128:(g + 1) * 128, pl.ds(q0, QB)]
            cols = []
            for j in js:
                parts = []
                if j > 0:
                    parts.append(jnp.zeros((j * SLOT, QB), BF16))
                parts.append(qg[j * SLOT:(j + 1) * SLOT])
                if j < GPH - 1:
                    parts.append(jnp.zeros((128 - (j + 1) * SLOT, QB), BF16))
                cols.append(jnp.concatenate(parts, axis=0))
            return _dot(kg, jnp.concatenate(cols, axis=1))

        def a_finish(q0, h, s):
            s0, s1, s2 = s[0:QB], s[QB:2 * QB], s[2 * QB:3 * QB]
            c = jnp.where(upper, s0, s2)
            m = jnp.maximum(jnp.max(c, axis=0, keepdims=True), jnp.max(s1, axis=0, keepdims=True))
            pc = jnp.exp2(c - m)
            p1 = jnp.exp2(s1 - m)
            p = jnp.concatenate([jnp.where(upper, pc, 0.0), p1, jnp.where(upper, 0.0, pc)], axis=0)
            vh = vT[h * SLOT:(h + 1) * SLOT, pl.ds(q0, 3 * QB)]
            o = _dot(vh, p.astype(BF16))
            return o * (1.0 / o[DHA:DHA + 1, :])

        def a_out(q0, oTs):
            oT = jnp.concatenate(oTs, axis=0)
            aT = _dot(woTp[...], oT.astype(BF16))
            aT = aT.astype(BF16).astype(F32)
            gaT[:, pl.ds(q0, QB)] = aT * gl[0:1, pl.ds(q0, QB)]

        rowE = lax.broadcasted_iota(jnp.int32, (32, 48), 0)
        colE = lax.broadcasted_iota(jnp.int32, (32, 48), 1)
        validE = (colE < M + SEG) & ((colE <= rowE) | (rowE < M))
        capE = jnp.where(validE, jnp.inf, NEG).astype(F32)
        rowO = lax.broadcasted_iota(jnp.int32, (48, 80), 0)
        colO = lax.broadcasted_iota(jnp.int32, (48, 80), 1)
        rtok = jnp.where(rowO < 32, rowO + 32, rowO - 8)
        ktok = jnp.where(colO < 48, colO - 8, colO - 16)
        k_m0 = colO < M
        k_m1 = (colO >= 48) & (colO < 48 + M)
        k_tok = jnp.logical_not(k_m0 | k_m1)
        r_mem = rowO < M
        r_seg1 = r_mem | (rtok >= SEG)
        validO = ((r_seg1 & (k_m1 | (k_tok & (ktok >= SEG) & ((ktok <= rtok) | r_mem)))) |
                  (jnp.logical_not(r_seg1) & (k_m0 | (k_tok & (ktok <= rtok)))))
        capO = jnp.where(validO, jnp.inf, NEG).astype(F32)

        def softmax_p(s, cap):
            s = jnp.minimum(s, cap)
            m = jnp.max(s, axis=-1, keepdims=True)
            e = jnp.exp2((s - m) * cexp_b)
            l = jnp.sum(e, axis=-1, keepdims=True)
            return e * (1.0 / l)

        def seg_step(hq, hin, prev, cap, hooks, ls, lp, nfill):
            qq = [None] * HB
            kv = [None] * HB
            p = [None] * HB
            v = [None] * HB
            o = [None] * HB

            def do_qkv(h):
                wq = pltpu.bitcast(wpk[:, h * 3 * E:h * 3 * E + E], BF16)
                wkv = pltpu.bitcast(wpk[:, h * 3 * E + E:(h + 1) * 3 * E], BF16)
                if QFIRST:
                    qq[h] = _dot(hq, wq)
                    kv[h] = _dot(hin, wkv)
                else:
                    kv[h] = _dot(hin, wkv)
                    qq[h] = _dot(hq, wq)

            def do_s(h):
                r = kv[h]
                if prev is None:
                    k, v[h] = r[:, :E], r[:, E:]
                else:
                    a = prev[h]
                    k = jnp.concatenate([a[:, :E], r[:, :E]], axis=0)
                    v[h] = jnp.concatenate([a[:, E:], r[:, E:]], axis=0)
                p[h] = softmax_p(_dot_nt(qq[h].astype(BF16), k.astype(BF16)), cap)

            def do_pv(h):
                o[h] = _dot(p[h].astype(BF16), v[h].astype(BF16))

            for t in range(HB):
                do_qkv(t)
                if t >= ls:
                    do_s(t - ls)
                if t >= lp:
                    do_pv(t - lp)
                if t in hooks:
                    hooks[t]()
            acc = None
            wo_next = 0
            for t in range(HB, HB + lp):
                for _ in range(nfill):
                    if wo_next < t - lp:
                        r = _dot(o[wo_next].astype(BF16), wob[wo_next * E:(wo_next + 1) * E, :])
                        acc = r if acc is None else acc + r
                        if ("wo", wo_next) in hooks:
                            hooks[("wo", wo_next)]()
                        wo_next += 1
                if t - ls < HB:
                    do_s(t - ls)
                do_pv(t - lp)
            for h in range(wo_next, HB):
                r = _dot(o[h].astype(BF16), wob[h * E:(h + 1) * E, :])
                acc = r if acc is None else acc + r
                if ("wo", h) in hooks:
                    hooks[("wo", h)]()
            if "end" in hooks:
                hooks["end"]()
            return acc, kv

        def pair(base, mem, hooksA, hooksB):
            t8 = xb[pl.ds(base, 8), :].astype(F32)
            g0 = jnp.concatenate([mem, t8], axis=0).astype(BF16)
            g12 = xb[pl.ds(base + 8, 32), :]
            hA = jnp.concatenate([g0, g12], axis=0)
            resA, kvA = seg_step(hA[0:32], hA, None, capE, hooksA, *LAG_E)
            mem1 = resA[0:8].astype(BF16).astype(F32)
            t8b = xb[pl.ds(base + 40, 8), :].astype(F32)
            g0b = jnp.concatenate([mem1, t8b], axis=0).astype(BF16)
            g1b = xb[pl.ds(base + 48, 16), :]
            hB = jnp.concatenate([g0b, g1b], axis=0)
            hQ = jnp.concatenate([hB, hA[32:48]], axis=0)
            resB, _ = seg_step(hQ, hB, kvA, capO, hooksB, *LAG_O)
            mem2 = resB[0:8].astype(BF16).astype(F32)
            b64 = jnp.concatenate([resA[8:32], resB[32:48], resB[8:32]], axis=0)
            bb[pl.ds(base, 64), :] = b64.astype(BF16)
            return mem2

        def super_iter(j, mem):
            q0 = pl.multiple_of(j * QB, QB)
            sc = {}
            oTs = [None] * HA

            def mk_scores(g, js):
                def f():
                    r = a_scores(q0, g, js)
                    for n, jj in enumerate(js):
                        sc[g * GPH + jj] = r[:, n * QB:(n + 1) * QB]
                return f

            def mk_finish(g, jj):
                def f():
                    oTs[g * GPH + jj] = a_finish(q0, g * GPH + jj, sc[g * GPH + jj])
                return f

            def hooks_for(g):
                hk = {}

                def add(t, f):
                    if t in hk:
                        g0_ = hk[t]
                        hk[t] = lambda: (g0_(), f())
                    else:
                        hk[t] = f
                for jj in range(GPH):
                    add(FIN_T[jj], mk_finish(g, jj))
                if SPLIT_S:
                    add(S2_T, mk_scores(g, (2, 3)))
                first = (0, 1) if SPLIT_S else (0, 1, 2, 3)
                if g + 1 < NG:
                    add(S_POS[g % 2], mk_scores(g + 1, first))
                else:
                    add(AOUT_T, lambda: a_out(q0, oTs))

                    def next_scores():
                        qn = pl.multiple_of(jnp.minimum(j + 1, NQB - 1) * QB, QB)
                        s0buf[...] = a_scores(qn, 0, (0, 1, 2, 3))
                    add(NS_POS, next_scores)
                return hk
            s0 = s0buf[...]
            for jj in range(GPH):
                sc[jj] = s0[:, jj * QB:(jj + 1) * QB]
            hk = [hooks_for(g) for g in range(NG)]
            prev = hk[0].get(COMB_T)

            def comb():
                if prev is not None:
                    prev()
                combine(pl.multiple_of(jnp.maximum(j - 1, 0) * QB, QB))
            hk[0][COMB_T] = comb
            mem = pair(q0, mem, hk[0], hk[1])
            mem = pair(q0 + 64, mem, hk[2], hk[3])

            @pl.when(j > 0)
            def _():
                out_copy(j - 1).start()
            return mem

        def combine(c0):
            bT = bb[pl.ds(c0, QB), :].T.astype(F32)
            g = gl[0:1, pl.ds(c0, QB)]
            outT[:, pl.ds(c0, QB)] = (gaT[:, pl.ds(c0, QB)] + (1.0 - g) * bT).astype(BF16)

        def out_copy(b):
            c0 = pl.multiple_of(b * QB, QB)
            return pltpu.make_async_copy(outT.at[:, pl.ds(c0, QB)], outT_hbm.at[:, pl.ds(c0, QB)], sems.at[16 + b])

        s0buf[...] = a_scores(0, 0, (0, 1, 2, 3))
        lax.fori_loop(0, NQB, super_iter, mem0_ref[...].astype(F32))
        combine((NQB - 1) * QB)
        out_copy(NQB - 1).start()
        for b in range(NQB):
            out_copy(b).wait()

    return kernel


@functools.partial(jax.jit, static_argnames=("B_seg_len",))
def pallas_gated_mix__sliding_block__memory_aug_recurrent_mem_tr__prompt_kernel(A_x, A_wqkv, A_wo, B_x, B_mem0, B_Wq, B_Wk, B_Wv, B_Wo, B_seg_len, gate_w):
    Bn, S, D = A_x.shape
    assert Bn == 1
    HB, E = B_Wq.shape[1], B_Wq.shape[2]
    M = B_mem0.shape[1]
    HA, WIN = 16, 256
    kern = _make_kernel(S, D, HA, WIN, HB, E, M, B_seg_len)
    hbm_spec = pl.BlockSpec(memory_space=pltpu.MemorySpace.HBM)
    vmem_spec = pl.BlockSpec(memory_space=pltpu.VMEM)
    outT = pl.pallas_call(
        kern,
        out_shape=jax.ShapeDtypeStruct((D, S), BF16),
        in_specs=[hbm_spec] * 9,
        out_specs=hbm_spec,
        scratch_shapes=[
            pltpu.VMEM((D, S), BF16),
            pltpu.VMEM((D, 3 * D), BF16),
            pltpu.VMEM((D, D), BF16),
            pltpu.VMEM((S, D), BF16),
            pltpu.VMEM((12, D * HB // 4, 128), U32),
            pltpu.VMEM((D // 2, 3 * HB * E), U32),
            pltpu.VMEM((HB * D, E), BF16),
            pltpu.VMEM((HB * E, D), BF16),
            pltpu.VMEM((3 * D + 16, D), BF16),
            pltpu.VMEM((D, 512), BF16),
            pltpu.VMEM((512, S), BF16),
            pltpu.VMEM((WIN + S, 512), BF16),
            pltpu.VMEM((512, WIN + S), BF16),
            pltpu.VMEM((8, S), F32),
            pltpu.VMEM((D, S), F32),
            pltpu.VMEM((S, D), BF16),
            pltpu.VMEM((D, S), BF16),
            pltpu.VMEM((3 * 128, 512), F32),
            pltpu.VMEM((M, D), BF16),
            pltpu.VMEM((D,), BF16),
            pltpu.SemaphoreType.DMA((38,)),
        ],
        compiler_params=pltpu.CompilerParams(vmem_limit_bytes=110 * 1024 * 1024),
    )(A_x.reshape(S, D).T, A_wqkv, A_wo, B_mem0.reshape(M, D),
      B_Wq.reshape(D // 2, 2 * HB, E), B_Wk.reshape(D // 2, 2 * HB, E), B_Wv.reshape(D // 2, 2 * HB, E),
      jnp.transpose(B_Wo, (0, 2, 1)).reshape(HB * D, E), gate_w)
    return outT.T.reshape(1, S, D)
```

```python
import functools
import math

import jax
import jax.numpy as jnp
from jax import lax
from jax.experimental import pallas as pl
from jax.experimental.pallas import tpu as pltpu

F32 = jnp.float32
BF16 = jnp.bfloat16
U32 = jnp.uint32
LOG2E = math.log2(math.e)
NEG = -1e9

NT = (((1,), (1,)), ((), ()))

DMA_ORDER = (("w", 0, 0), ("wo", 0), ("w", 0, 1), ("w", 1, 0), ("wo", 1), ("w", 1, 1), ("wo", 2), ("wo", 3),
             ("w", 2, 0), ("w", 2, 1))
FIN_T = (5, 7, 9, 11)
AOUT_T = 14
COMB_T = 2
LAG_E = (1, 3, 3)
LAG_O = (2, 4, 2)


def _dot(a, b):
    return jnp.dot(a, b, preferred_element_type=F32)


def _dot_nt(a, b):
    return lax.dot_general(a, b, NT, preferred_element_type=F32)


def _bf16_round(v):
    m, e = math.frexp(v)
    return math.ldexp(round(m * 256.0) / 256.0, e)


def _make_kernel(S, D, HA, W, HB, E, M, SEG):
    DHA = D // HA
    SLOT = 32
    DP = HA * SLOT
    QB = 128
    NQB = S // QB
    GPH = 128 // SLOT
    NG = HA // GPH
    PCH = 256
    NPC = S // PCH
    NP1 = 3
    NWO = 4
    HPW = HB // NWO
    HH = HB // 2
    assert SEG == 32 and M == 8 and W == 2 * QB and D % 16 == 0 and DHA < SLOT
    assert NPC - NP1 == 5 and NG == 4 and E == 256 and HB == 16
    cexp_a = _bf16_round(DHA ** -0.5) * LOG2E
    cexp_b = _bf16_round(E ** -0.5) * LOG2E

    def kernel(xaT_hbm, wqkv_hbm, wo_hbm, mem0_hbm, wq_hbm, wk_hbm, wv_hbm, woT_hbm, gate_hbm,
               outT_hbm,
               xaT, wqkv, wo, xb, wraw, wpk, woTraw, wob, wTp, woTp, qT, kk, vT, gl, gaT, bb, outT, s0buf,
               mem0_ref, gate_ref, sems):
        cps = {}

        def start(name, src, dst, idx):
            cp = pltpu.make_async_copy(src, dst, sems.at[idx])
            cp.start()
            cps[name] = cp
        start("wqkv", wqkv_hbm, wqkv, 0)
        start("gate", gate_hbm, gate_ref, 32)
        start("mem0", mem0_hbm, mem0_ref, 33)
        start("xa", xaT_hbm, xaT, 1)
        start("wo", wo_hbm, wo, 2)

        def w_copy(mi, t, par):
            wu = (wq_hbm, wk_hbm, wv_hbm)[mi].bitcast(U32)
            dst = wraw.at[(mi * 2 + t) * 2 + par].reshape(D // 2, HH, 128)
            return pltpu.make_async_copy(wu.at[:, par * HH:(par + 1) * HH, t * 128:(t + 1) * 128],
                                         dst, sems.at[4 + (mi * 2 + t) * 2 + par])

        def w_wait(mi, t):
            for par in range(2):
                w_copy(mi, t, par).wait()

        def wo_copy(k):
            r0 = k * HPW * D
            return pltpu.make_async_copy(woT_hbm.at[pl.ds(r0, HPW * D)], woTraw.at[pl.ds(r0, HPW * D)],
                                         sems.at[34 + k])

        for item in DMA_ORDER:
            if item[0] == "w":
                for par in range(2):
                    w_copy(item[1], item[2], par).start()
            else:
                wo_copy(item[1]).start()

        cps["wqkv"].wait()

        def respace(r, fill):
            n = r.shape[1]
            first = lax.broadcasted_iota(jnp.int32, (SLOT - DHA, n), 0) == 0
            pad = jnp.where(first, fill, 0.0).astype(r.dtype)
            parts = []
            for h in range(HA):
                parts += [r[h * DHA:(h + 1) * DHA], pad]
            return jnp.concatenate(parts, axis=0)

        wTp[0:3 * D, :] = wqkv[...].T
        cps["gate"].wait()
        cps["mem0"].wait()
        wTp[3 * D:3 * D + 16, :] = jnp.broadcast_to(gate_ref[...].reshape(1, D), (16, D))
        cps["wo"].wait()
        woTp[...] = respace(wo[...].astype(F32), 0.0).T.astype(BF16)
        lane = lax.broadcasted_iota(jnp.int32, (W, DP), 1)
        kk[0:W, :] = jnp.where(lane % SLOT == DHA, NEG, 0.0).astype(BF16)
        vT[:, 0:W] = jnp.zeros((DP, W), BF16)
        gaT[:, 0:QB] = jnp.zeros((D, QB), F32)
        bb[0:QB, :] = jnp.zeros((QB, D), BF16)

        cps["xa"].wait()

        def proj(c):
            col = pl.multiple_of(c * PCH, PCH)
            xc = xaT[:, pl.ds(col, PCH)]
            qT[:, pl.ds(col, PCH)] = respace(_dot(wTp[0:D, :], xc) * cexp_a, 1.0).astype(BF16)
            kk[pl.ds(W + col, PCH), :] = respace(_dot(wTp[D:2 * D, :], xc), 0.0).astype(BF16).T
            r = _dot(wTp[2 * D:3 * D + 16, :], xc)
            vT[:, pl.ds(W + col, PCH)] = respace(r[0:D], 1.0).astype(BF16)
            gl[:, pl.ds(col, PCH)] = jax.nn.sigmoid(r[D:D + 8])
            xb[pl.ds(col, PCH), :] = xc.T

        def wob_head(h):
            wob[pl.ds(pl.multiple_of(h * E, E), E), :] = woTraw[pl.ds(pl.multiple_of(h * D, 16), D), :].T

        def w_unit(u):
            mt = u // HH
            j = u % HH
            mi = mt // 2
            t = mt % 2
            xe = wraw[2 * mt, pl.ds(j, D // 2, stride=HH), :]
            xo = wraw[2 * mt + 1, pl.ds(j, D // 2, stride=HH), :]
            lo = (xe & U32(0xFFFF)) | (xo << 16)
            hi = (xe >> 16) | (xo & U32(0xFFFF0000))
            c0 = pl.multiple_of((2 * j) * 3 * E + mi * E + t * 128, 128)
            wpk[:, pl.ds(c0, 128)] = lo
            wpk[:, pl.ds(c0 + 3 * E, 128)] = hi

        def p1(c, carry):
            proj(c)
            return carry
        lax.fori_loop(0, NP1, p1, 0)

        def p3(c, carry):
            for n in range(NPC - NP1):
                @pl.when(c == NP1 + n)
                def _():
                    w_wait(n // 2, n % 2)
                    if n == 0:
                        wo_copy(0).wait()
                    elif n >= 2:
                        wo_copy(n - 1).wait()
            proj(c)
            for k in range(HH):
                w_unit((c - NP1) * HH + k)
            piece = jnp.maximum(c - NP1 - 1, 0)
            for n in range(HPW):
                wob_head(piece * HPW + n)
            return carry
        lax.fori_loop(NP1, NPC, p3, 0)
        w_wait(2, 1)

        def p4(u, carry):
            w_unit(5 * HH + 2 * u)
            w_unit(5 * HH + 2 * u + 1)
            return carry
        lax.fori_loop(0, HH // 2, p4, 0)

        krow = lax.broadcasted_iota(jnp.int32, (QB, QB), 0)
        qcol = lax.broadcasted_iota(jnp.int32, (QB, QB), 1)
        upper = krow > qcol

        def a_scores(q0, g):
            kg = kk[pl.ds(q0, 3 * QB), g * 128:(g + 1) * 128]
            qg = qT[g * 128:(g + 1) * 128, pl.ds(q0, QB)]
            cols = []
            for j in range(GPH):
                parts = []
                if j > 0:
                    parts.append(jnp.zeros((j * SLOT, QB), BF16))
                parts.append(qg[j * SLOT:(j + 1) * SLOT])
                if j < GPH - 1:
                    parts.append(jnp.zeros((128 - (j + 1) * SLOT, QB), BF16))
                cols.append(jnp.concatenate(parts, axis=0))
            return _dot(kg, jnp.concatenate(cols, axis=1))

        def a_finish(q0, h, s):
            s0, s1, s2 = s[0:QB], s[QB:2 * QB], s[2 * QB:3 * QB]
            c = jnp.where(upper, s0, s2)
            m = jnp.maximum(jnp.max(c, axis=0, keepdims=True), jnp.max(s1, axis=0, keepdims=True))
            pc = jnp.exp2(c - m)
            p1_ = jnp.exp2(s1 - m)
            p = jnp.concatenate([jnp.where(upper, pc, 0.0), p1_, jnp.where(upper, 0.0, pc)], axis=0)
            vh = vT[h * SLOT:(h + 1) * SLOT, pl.ds(q0, 3 * QB)]
            o = _dot(vh, p.astype(BF16))
            return o * (1.0 / o[DHA:DHA + 1, :])

        def a_out(q0, oTs):
            oT = jnp.concatenate(oTs, axis=0)
            aT = _dot(woTp[...], oT.astype(BF16))
            aT = aT.astype(BF16).astype(F32)
            gaT[:, pl.ds(q0, QB)] = aT * gl[0:1, pl.ds(q0, QB)]

        rowE = lax.broadcasted_iota(jnp.int32, (32, 48), 0)
        colE = lax.broadcasted_iota(jnp.int32, (32, 48), 1)
        validE = (colE < M + SEG) & ((colE <= rowE) | (rowE < M))
        capE = jnp.where(validE, jnp.inf, NEG).astype(F32)
        rowO = lax.broadcasted_iota(jnp.int32, (48, 80), 0)
        colO = lax.broadcasted_iota(jnp.int32, (48, 80), 1)
        rtok = jnp.where(rowO < 32, rowO + 32, rowO - 8)
        ktok = jnp.where(colO < 48, colO - 8, colO - 16)
        k_m0 = colO < M
        k_m1 = (colO >= 48) & (colO < 48 + M)
        k_tok = jnp.logical_not(k_m0 | k_m1)
        r_mem = rowO < M
        r_seg1 = r_mem | (rtok >= SEG)
        validO = ((r_seg1 & (k_m1 | (k_tok & (ktok >= SEG) & ((ktok <= rtok) | r_mem)))) |
                  (jnp.logical_not(r_seg1) & (k_m0 | (k_tok & (ktok <= rtok)))))
        capO = jnp.where(validO, jnp.inf, NEG).astype(F32)

        def softmax_p(s, cap):
            s = jnp.minimum(s, cap)
            m = jnp.max(s, axis=-1, keepdims=True)
            e = jnp.exp2((s - m) * cexp_b)
            l = jnp.sum(e, axis=-1, keepdims=True)
            return e * (1.0 / l)

        def seg_step(hq, hin, prev, cap, hooks, ls, lp, nfill):
            qq = [None] * HB
            kv = [None] * HB
            p = [None] * HB
            v = [None] * HB
            o = [None] * HB

            def do_qkv(h):
                wq = pltpu.bitcast(wpk[:, h * 3 * E:h * 3 * E + E], BF16)
                wkv = pltpu.bitcast(wpk[:, h * 3 * E + E:(h + 1) * 3 * E], BF16)
                kv[h] = _dot(hin, wkv)
                qq[h] = _dot(hq, wq)

            def do_s(h):
                r = kv[h]
                if prev is None:
                    k, v[h] = r[:, :E], r[:, E:]
                else:
                    a = prev[h]
                    k = jnp.concatenate([a[:, :E], r[:, :E]], axis=0)
                    v[h] = jnp.concatenate([a[:, E:], r[:, E:]], axis=0)
                p[h] = softmax_p(_dot_nt(qq[h].astype(BF16), k.astype(BF16)), cap)

            def do_pv(h):
                o[h] = _dot(p[h].astype(BF16), v[h].astype(BF16))

            def do_wo(h, acc):
                r = _dot(o[h].astype(BF16), wob[h * E:(h + 1) * E, :])
                return r if acc is None else acc + r

            for t in range(HB):
                do_qkv(t)
                if t >= ls:
                    do_s(t - ls)
                if t >= lp:
                    do_pv(t - lp)
                for f in hooks.get(t, ()):
                    f()
            acc = None
            wo_next = 0
            for t in range(HB, HB + lp):
                for _ in range(nfill):
                    if wo_next < t - lp:
                        acc = do_wo(wo_next, acc)
                        wo_next += 1
                if t - ls < HB:
                    do_s(t - ls)
                do_pv(t - lp)
            for h in range(wo_next, HB):
                acc = do_wo(h, acc)
            for f in hooks.get("end", ()):
                f()
            return acc, kv

        def pair(base, mem, hooksE, hooksO):
            t8 = xb[pl.ds(base, 8), :].astype(F32)
            g0 = jnp.concatenate([mem, t8], axis=0).astype(BF16)
            g12 = xb[pl.ds(base + 8, 32), :]
            hA = jnp.concatenate([g0, g12], axis=0)
            resA, kvA = seg_step(hA[0:32], hA, None, capE, hooksE, *LAG_E)
            mem1 = resA[0:8].astype(BF16).astype(F32)
            t8b = xb[pl.ds(base + 40, 8), :].astype(F32)
            g0b = jnp.concatenate([mem1, t8b], axis=0).astype(BF16)
            g1b = xb[pl.ds(base + 48, 16), :]
            hB = jnp.concatenate([g0b, g1b], axis=0)
            hQ = jnp.concatenate([hB, hA[32:48]], axis=0)
            resB, _ = seg_step(hQ, hB, kvA, capO, hooksO, *LAG_O)
            mem2 = resB[0:8].astype(BF16).astype(F32)
            b64 = jnp.concatenate([resA[8:32], resB[32:48], resB[8:32]], axis=0)
            bb[pl.ds(base, 64), :] = b64.astype(BF16)
            return mem2

        def combine(c0):
            bT = bb[pl.ds(c0, QB), :].T.astype(F32)
            g = gl[0:1, pl.ds(c0, QB)]
            outT[:, pl.ds(c0, QB)] = (gaT[:, pl.ds(c0, QB)] + (1.0 - g) * bT).astype(BF16)

        def out_copy(b):
            c0 = pl.multiple_of(b * QB, QB)
            return pltpu.make_async_copy(outT.at[:, pl.ds(c0, QB)], outT_hbm.at[:, pl.ds(c0, QB)], sems.at[16 + b])

        def super_iter(j, mem):
            q0 = pl.multiple_of(j * QB, QB)
            sc = {}
            oTs = [None] * HA

            def keep_scores(g, r):
                for jj in range(GPH):
                    sc[g * GPH + jj] = r[:, jj * QB:(jj + 1) * QB]

            def finish(h):
                oTs[h] = a_finish(q0, h, sc[h])

            def next_scores():
                qn = pl.multiple_of(jnp.minimum(j + 1, NQB - 1) * QB, QB)
                s0buf[...] = a_scores(qn, 0)

            hk = []
            for g in range(NG):
                h_g = {}
                for jj in range(GPH):
                    h_g.setdefault(FIN_T[jj], []).append(functools.partial(finish, g * GPH + jj))
                if g + 1 < NG:
                    h_g["end"] = [lambda g=g: keep_scores(g + 1, a_scores(q0, g + 1))]
                else:
                    h_g.setdefault(AOUT_T, []).append(lambda: a_out(q0, oTs))
                    h_g["end"] = [next_scores]
                hk.append(h_g)
            hk[0].setdefault(COMB_T, []).append(
                lambda: combine(pl.multiple_of(jnp.maximum(j - 1, 0) * QB, QB)))

            keep_scores(0, s0buf[...])
            mem = pair(q0, mem, hk[0], hk[1])
            mem = pair(q0 + 64, mem, hk[2], hk[3])

            @pl.when(j > 0)
            def _():
                out_copy(j - 1).start()
            return mem

        s0buf[...] = a_scores(0, 0)
        lax.fori_loop(0, NQB, super_iter, mem0_ref[...].astype(F32))
        combine((NQB - 1) * QB)
        out_copy(NQB - 1).start()
        for b in range(NQB):
            out_copy(b).wait()

    return kernel


@functools.partial(jax.jit, static_argnames=("B_seg_len",))
def pallas_gated_mix__sliding_block__memory_aug_recurrent_mem_tr__prompt_kernel(
        A_x, A_wqkv, A_wo, B_x, B_mem0, B_Wq, B_Wk, B_Wv, B_Wo, B_seg_len, gate_w):
    del B_x
    Bn, S, D = A_x.shape
    assert Bn == 1
    HB, E = B_Wq.shape[1], B_Wq.shape[2]
    M = B_mem0.shape[1]
    HA, WIN = 16, 256
    kern = _make_kernel(S, D, HA, WIN, HB, E, M, B_seg_len)
    hbm_spec = pl.BlockSpec(memory_space=pltpu.MemorySpace.HBM)
    outT = pl.pallas_call(
        kern,
        out_shape=jax.ShapeDtypeStruct((D, S), BF16),
        in_specs=[hbm_spec] * 9,
        out_specs=hbm_spec,
        scratch_shapes=[
            pltpu.VMEM((D, S), BF16),
            pltpu.VMEM((D, 3 * D), BF16),
            pltpu.VMEM((D, D), BF16),
            pltpu.VMEM((S, D), BF16),
            pltpu.VMEM((12, D * HB // 4, 128), U32),
            pltpu.VMEM((D // 2, 3 * HB * E), U32),
            pltpu.VMEM((HB * D, E), BF16),
            pltpu.VMEM((HB * E, D), BF16),
            pltpu.VMEM((3 * D + 16, D), BF16),
            pltpu.VMEM((D, 512), BF16),
            pltpu.VMEM((512, S), BF16),
            pltpu.VMEM((WIN + S, 512), BF16),
            pltpu.VMEM((512, WIN + S), BF16),
            pltpu.VMEM((8, S), F32),
            pltpu.VMEM((D, S), F32),
            pltpu.VMEM((S, D), BF16),
            pltpu.VMEM((D, S), BF16),
            pltpu.VMEM((3 * 128, 512), F32),
            pltpu.VMEM((M, D), BF16),
            pltpu.VMEM((D,), BF16),
            pltpu.SemaphoreType.DMA((38,)),
        ],
        compiler_params=pltpu.CompilerParams(vmem_limit_bytes=110 * 1024 * 1024),
    )(A_x.reshape(S, D).T, A_wqkv, A_wo, B_mem0.reshape(M, D),
      B_Wq.reshape(D // 2, 2 * HB, E), B_Wk.reshape(D // 2, 2 * HB, E), B_Wv.reshape(D // 2, 2 * HB, E),
      jnp.transpose(B_Wo, (0, 2, 1)).reshape(HB * D, E), gate_w)
    return outT.T.reshape(1, S, D)
```

```python
import functools
import math

import jax
import jax.numpy as jnp
from jax import lax
from jax.experimental import pallas as pl
from jax.experimental.pallas import tpu as pltpu

F32 = jnp.float32
BF16 = jnp.bfloat16
U32 = jnp.uint32
LOG2E = math.log2(math.e)
NEG = -1e9

NT = (((1,), (1,)), ((), ()))

DMA_ORDER = (("w", 0, 0), ("wo", 0), ("w", 0, 1), ("w", 1, 0), ("wo", 1), ("w", 1, 1), ("wo", 2), ("wo", 3),
             ("w", 2, 0), ("w", 2, 1))
FIN_T = (5, 7, 9, 11)
AOUT_T = 14
COMB_T = 2
LAG_E = (1, 3, 3)
LAG_O = (2, 4, 2)


def _dot(a, b):
    return jnp.dot(a, b, preferred_element_type=F32)


def _dot_nt(a, b):
    return lax.dot_general(a, b, NT, preferred_element_type=F32)


def _bf16_round(v):
    m, e = math.frexp(v)
    return math.ldexp(round(m * 256.0) / 256.0, e)


def _make_kernel(S, D, HA, W, HB, E, M, SEG):
    DHA = D // HA
    SLOT = 32
    DP = HA * SLOT
    QB = 128
    NQB = S // QB
    GPH = 128 // SLOT
    NG = HA // GPH
    PCH = 256
    NPC = S // PCH
    NP1 = 3
    NWO = 4
    HPW = HB // NWO
    HH = HB // 2
    assert SEG == 32 and M == 8 and W == 2 * QB and D % 16 == 0 and DHA < SLOT
    assert NPC - NP1 == 5 and NG == 4 and E == 256 and HB == 16
    cexp_a = _bf16_round(DHA ** -0.5) * LOG2E
    cexp_b = _bf16_round(E ** -0.5) * LOG2E

    def kernel(xaT_hbm, wqkv_hbm, wo_hbm, mem0_hbm, wq_hbm, wk_hbm, wv_hbm, woT_hbm, gate_hbm,
               outT_hbm,
               xaT, wqkv, wo, xb, wraw, wpk, woTraw, wob, wTp, woTp, qT, kk, vT, gl, gaT, bb, outT, s0buf,
               mem0_ref, gate_ref, sems):
        cps = {}

        def start(name, src, dst, idx):
            cp = pltpu.make_async_copy(src, dst, sems.at[idx])
            cp.start()
            cps[name] = cp
        start("gate", gate_hbm, gate_ref, 32)
        start("mem0", mem0_hbm, mem0_ref, 33)
        start("wqkv", wqkv_hbm, wqkv, 0)

        def x_copy(c):
            col = pl.multiple_of(c * PCH, PCH)
            return pltpu.make_async_copy(xaT_hbm.at[:, pl.ds(col, PCH)], xaT.at[:, pl.ds(col, PCH)], sems.at[38 + c])
        for c in range(NPC):
            x_copy(c).start()
        start("wo", wo_hbm, wo, 2)

        def w_copy(mi, t, par):
            wu = (wq_hbm, wk_hbm, wv_hbm)[mi].bitcast(U32)
            dst = wraw.at[(mi * 2 + t) * 2 + par].reshape(D // 2, HH, 128)
            return pltpu.make_async_copy(wu.at[:, par * HH:(par + 1) * HH, t * 128:(t + 1) * 128],
                                         dst, sems.at[4 + (mi * 2 + t) * 2 + par])

        def w_wait(mi, t):
            for par in range(2):
                w_copy(mi, t, par).wait()

        def wo_copy(k):
            r0 = k * HPW * D
            return pltpu.make_async_copy(woT_hbm.at[pl.ds(r0, HPW * D)], woTraw.at[pl.ds(r0, HPW * D)],
                                         sems.at[34 + k])

        for item in DMA_ORDER:
            if item[0] == "w":
                for par in range(2):
                    w_copy(item[1], item[2], par).start()
            else:
                wo_copy(item[1]).start()

        lane = lax.broadcasted_iota(jnp.int32, (W, DP), 1)
        kk[0:W, :] = jnp.where(lane % SLOT == DHA, NEG, 0.0).astype(BF16)
        vT[:, 0:W] = jnp.zeros((DP, W), BF16)
        gaT[:, 0:QB] = jnp.zeros((D, QB), F32)
        bb[0:QB, :] = jnp.zeros((QB, D), BF16)

        def respace(r, fill):
            n = r.shape[1]
            first = lax.broadcasted_iota(jnp.int32, (SLOT - DHA, n), 0) == 0
            pad = jnp.where(first, fill, 0.0).astype(r.dtype)
            parts = []
            for h in range(HA):
                parts += [r[h * DHA:(h + 1) * DHA], pad]
            return jnp.concatenate(parts, axis=0)

        cps["gate"].wait()
        cps["mem0"].wait()
        wTp[3 * D:3 * D + 16, :] = jnp.broadcast_to(gate_ref[...].reshape(1, D), (16, D))
        cps["wqkv"].wait()
        wTp[0:3 * D, :] = wqkv[...].T

        def proj(c):
            x_copy(c).wait()
            col = pl.multiple_of(c * PCH, PCH)
            xc = xaT[:, pl.ds(col, PCH)]
            qT[:, pl.ds(col, PCH)] = respace(_dot(wTp[0:D, :], xc) * cexp_a, 1.0).astype(BF16)
            kk[pl.ds(W + col, PCH), :] = respace(_dot(wTp[D:2 * D, :], xc), 0.0).astype(BF16).T
            r = _dot(wTp[2 * D:3 * D + 16, :], xc)
            vT[:, pl.ds(W + col, PCH)] = respace(r[0:D], 1.0).astype(BF16)
            gl[:, pl.ds(col, PCH)] = jax.nn.sigmoid(r[D:D + 8])
            xb[pl.ds(col, PCH), :] = xc.T

        def wob_head(h):
            wob[pl.ds(pl.multiple_of(h * E, E), E), :] = woTraw[pl.ds(pl.multiple_of(h * D, 16), D), :].T

        def w_unit(u):
            mt = u // HH
            j = u % HH
            mi = mt // 2
            t = mt % 2
            xe = wraw[2 * mt, pl.ds(j, D // 2, stride=HH), :]
            xo = wraw[2 * mt + 1, pl.ds(j, D // 2, stride=HH), :]
            lo = (xe & U32(0xFFFF)) | (xo << 16)
            hi = (xe >> 16) | (xo & U32(0xFFFF0000))
            c0 = pl.multiple_of((2 * j) * 3 * E + mi * E + t * 128, 128)
            wpk[:, pl.ds(c0, 128)] = lo
            wpk[:, pl.ds(c0 + 3 * E, 128)] = hi

        def p1(c, carry):
            proj(c)
            return carry
        lax.fori_loop(0, NP1, p1, 0)
        cps["wo"].wait()
        woTp[...] = respace(wo[...].astype(F32), 0.0).T.astype(BF16)

        def p3(c, carry):
            for n in range(NPC - NP1):
                @pl.when(c == NP1 + n)
                def _():
                    w_wait(n // 2, n % 2)
                    if n == 0:
                        wo_copy(0).wait()
                    elif n >= 2:
                        wo_copy(n - 1).wait()
            proj(c)
            for k in range(HH):
                w_unit((c - NP1) * HH + k)
            piece = jnp.maximum(c - NP1 - 1, 0)
            for n in range(HPW):
                wob_head(piece * HPW + n)
            return carry
        lax.fori_loop(NP1, NPC, p3, 0)
        w_wait(2, 1)

        def p4(u, carry):
            w_unit(5 * HH + 2 * u)
            w_unit(5 * HH + 2 * u + 1)
            return carry
        lax.fori_loop(0, HH // 2, p4, 0)

        krow = lax.broadcasted_iota(jnp.int32, (QB, QB), 0)
        qcol = lax.broadcasted_iota(jnp.int32, (QB, QB), 1)
        upper = krow > qcol

        def a_scores(q0, g):
            kg = kk[pl.ds(q0, 3 * QB), g * 128:(g + 1) * 128]
            qg = qT[g * 128:(g + 1) * 128, pl.ds(q0, QB)]
            cols = []
            for j in range(GPH):
                parts = []
                if j > 0:
                    parts.append(jnp.zeros((j * SLOT, QB), BF16))
                parts.append(qg[j * SLOT:(j + 1) * SLOT])
                if j < GPH - 1:
                    parts.append(jnp.zeros((128 - (j + 1) * SLOT, QB), BF16))
                cols.append(jnp.concatenate(parts, axis=0))
            return _dot(kg, jnp.concatenate(cols, axis=1))

        def a_finish(q0, h, s):
            s0, s1, s2 = s[0:QB], s[QB:2 * QB], s[2 * QB:3 * QB]
            c = jnp.where(upper, s0, s2)
            m = jnp.maximum(jnp.max(c, axis=0, keepdims=True), jnp.max(s1, axis=0, keepdims=True))
            pc = jnp.exp2(c - m)
            p1_ = jnp.exp2(s1 - m)
            p = jnp.concatenate([jnp.where(upper, pc, 0.0), p1_, jnp.where(upper, 0.0, pc)], axis=0)
            vh = vT[h * SLOT:(h + 1) * SLOT, pl.ds(q0, 3 * QB)]
            o = _dot(vh, p.astype(BF16))
            return o * (1.0 / o[DHA:DHA + 1, :])

        def a_out(q0, oTs):
            oT = jnp.concatenate(oTs, axis=0)
            aT = _dot(woTp[...], oT.astype(BF16))
            aT = aT.astype(BF16).astype(F32)
            gaT[:, pl.ds(q0, QB)] = aT * gl[0:1, pl.ds(q0, QB)]

        rowE = lax.broadcasted_iota(jnp.int32, (32, 48), 0)
        colE = lax.broadcasted_iota(jnp.int32, (32, 48), 1)
        validE = (colE < M + SEG) & ((colE <= rowE) | (rowE < M))
        capE = jnp.where(validE, jnp.inf, NEG).astype(F32)
        rowO = lax.broadcasted_iota(jnp.int32, (48, 80), 0)
        colO = lax.broadcasted_iota(jnp.int32, (48, 80), 1)
        rtok = jnp.where(rowO < 32, rowO + 32, rowO - 8)
        ktok = jnp.where(colO < 48, colO - 8, colO - 16)
        k_m0 = colO < M
        k_m1 = (colO >= 48) & (colO < 48 + M)
        k_tok = jnp.logical_not(k_m0 | k_m1)
        r_mem = rowO < M
        r_seg1 = r_mem | (rtok >= SEG)
        validO = ((r_seg1 & (k_m1 | (k_tok & (ktok >= SEG) & ((ktok <= rtok) | r_mem)))) |
                  (jnp.logical_not(r_seg1) & (k_m0 | (k_tok & (ktok <= rtok)))))
        capO = jnp.where(validO, jnp.inf, NEG).astype(F32)

        def softmax_p(s, cap):
            s = jnp.minimum(s, cap)
            m = jnp.max(s, axis=-1, keepdims=True)
            e = jnp.exp2((s - m) * cexp_b)
            l = jnp.sum(e, axis=-1, keepdims=True)
            return e * (1.0 / l)

        def seg_step(hq, hin, prev, cap, hooks, ls, lp, nfill):
            qq = [None] * HB
            kv = [None] * HB
            p = [None] * HB
            v = [None] * HB
            o = [None] * HB

            def do_qkv(h):
                wq = pltpu.bitcast(wpk[:, h * 3 * E:h * 3 * E + E], BF16)
                wkv = pltpu.bitcast(wpk[:, h * 3 * E + E:(h + 1) * 3 * E], BF16)
                kv[h] = _dot(hin, wkv)
                qq[h] = _dot(hq, wq)

            def do_s(h):
                r = kv[h]
                if prev is None:
                    k, v[h] = r[:, :E], r[:, E:]
                else:
                    a = prev[h]
                    k = jnp.concatenate([a[:, :E], r[:, :E]], axis=0)
                    v[h] = jnp.concatenate([a[:, E:], r[:, E:]], axis=0)
                p[h] = softmax_p(_dot_nt(qq[h].astype(BF16), k.astype(BF16)), cap)

            def do_pv(h):
                o[h] = _dot(p[h].astype(BF16), v[h].astype(BF16))

            def do_wo(h, acc):
                r = _dot(o[h].astype(BF16), wob[h * E:(h + 1) * E, :])
                return r if acc is None else acc + r

            for t in range(HB):
                do_qkv(t)
                if t >= ls:
                    do_s(t - ls)
                if t >= lp:
                    do_pv(t - lp)
                for f in hooks.get(t, ()):
                    f()
            acc = None
            wo_next = 0
            for t in range(HB, HB + lp):
                for _ in range(nfill):
                    if wo_next < t - lp:
                        acc = do_wo(wo_next, acc)
                        wo_next += 1
                if t - ls < HB:
                    do_s(t - ls)
                do_pv(t - lp)
            for h in range(wo_next, HB):
                acc = do_wo(h, acc)
            for f in hooks.get("end", ()):
                f()
            return acc, kv

        def pair(base, mem, hooksE, hooksO):
            t8 = xb[pl.ds(base, 8), :].astype(F32)
            g0 = jnp.concatenate([mem, t8], axis=0).astype(BF16)
            g12 = xb[pl.ds(base + 8, 32), :]
            hA = jnp.concatenate([g0, g12], axis=0)
            resA, kvA = seg_step(hA[0:32], hA, None, capE, hooksE, *LAG_E)
            mem1 = resA[0:8].astype(BF16).astype(F32)
            t8b = xb[pl.ds(base + 40, 8), :].astype(F32)
            g0b = jnp.concatenate([mem1, t8b], axis=0).astype(BF16)
            g1b = xb[pl.ds(base + 48, 16), :]
            hB = jnp.concatenate([g0b, g1b], axis=0)
            hQ = jnp.concatenate([hB, hA[32:48]], axis=0)
            resB, _ = seg_step(hQ, hB, kvA, capO, hooksO, *LAG_O)
            mem2 = resB[0:8].astype(BF16).astype(F32)
            b64 = jnp.concatenate([resA[8:32], resB[32:48], resB[8:32]], axis=0)
            bb[pl.ds(base, 64), :] = b64.astype(BF16)
            return mem2

        def combine(c0):
            bT = bb[pl.ds(c0, QB), :].T.astype(F32)
            g = gl[0:1, pl.ds(c0, QB)]
            outT[:, pl.ds(c0, QB)] = (gaT[:, pl.ds(c0, QB)] + (1.0 - g) * bT).astype(BF16)

        def out_copy(b):
            c0 = pl.multiple_of(b * QB, QB)
            return pltpu.make_async_copy(outT.at[:, pl.ds(c0, QB)], outT_hbm.at[:, pl.ds(c0, QB)], sems.at[16 + b])

        def super_iter(j, mem):
            q0 = pl.multiple_of(j * QB, QB)
            sc = {}
            oTs = [None] * HA

            def keep_scores(g, r):
                for jj in range(GPH):
                    sc[g * GPH + jj] = r[:, jj * QB:(jj + 1) * QB]

            def finish(h):
                oTs[h] = a_finish(q0, h, sc[h])

            def next_scores():
                qn = pl.multiple_of(jnp.minimum(j + 1, NQB - 1) * QB, QB)
                s0buf[...] = a_scores(qn, 0)

            hk = []
            for g in range(NG):
                h_g = {}
                for jj in range(GPH):
                    h_g.setdefault(FIN_T[jj], []).append(functools.partial(finish, g * GPH + jj))
                if g + 1 < NG:
                    h_g["end"] = [lambda g=g: keep_scores(g + 1, a_scores(q0, g + 1))]
                else:
                    h_g.setdefault(AOUT_T, []).append(lambda: a_out(q0, oTs))
                    h_g["end"] = [next_scores]
                hk.append(h_g)
            hk[0].setdefault(COMB_T, []).append(
                lambda: combine(pl.multiple_of(jnp.maximum(j - 1, 0) * QB, QB)))

            keep_scores(0, s0buf[...])
            mem = pair(q0, mem, hk[0], hk[1])
            mem = pair(q0 + 64, mem, hk[2], hk[3])

            @pl.when(j > 0)
            def _():
                out_copy(j - 1).start()
            return mem

        s0buf[...] = a_scores(0, 0)
        lax.fori_loop(0, NQB, super_iter, mem0_ref[...].astype(F32))
        combine((NQB - 1) * QB)
        out_copy(NQB - 1).start()
        for b in range(NQB):
            out_copy(b).wait()

    return kernel


@functools.partial(jax.jit, static_argnames=("B_seg_len",))
def pallas_gated_mix__sliding_block__memory_aug_recurrent_mem_tr__prompt_kernel(
        A_x, A_wqkv, A_wo, B_x, B_mem0, B_Wq, B_Wk, B_Wv, B_Wo, B_seg_len, gate_w):
    del B_x
    Bn, S, D = A_x.shape
    assert Bn == 1
    HB, E = B_Wq.shape[1], B_Wq.shape[2]
    M = B_mem0.shape[1]
    HA, WIN = 16, 256
    kern = _make_kernel(S, D, HA, WIN, HB, E, M, B_seg_len)
    hbm_spec = pl.BlockSpec(memory_space=pltpu.MemorySpace.HBM)
    outT = pl.pallas_call(
        kern,
        out_shape=jax.ShapeDtypeStruct((D, S), BF16),
        in_specs=[hbm_spec] * 9,
        out_specs=hbm_spec,
        scratch_shapes=[
            pltpu.VMEM((D, S), BF16),
            pltpu.VMEM((D, 3 * D), BF16),
            pltpu.VMEM((D, D), BF16),
            pltpu.VMEM((S, D), BF16),
            pltpu.VMEM((12, D * HB // 4, 128), U32),
            pltpu.VMEM((D // 2, 3 * HB * E), U32),
            pltpu.VMEM((HB * D, E), BF16),
            pltpu.VMEM((HB * E, D), BF16),
            pltpu.VMEM((3 * D + 16, D), BF16),
            pltpu.VMEM((D, 512), BF16),
            pltpu.VMEM((512, S), BF16),
            pltpu.VMEM((WIN + S, 512), BF16),
            pltpu.VMEM((512, WIN + S), BF16),
            pltpu.VMEM((8, S), F32),
            pltpu.VMEM((D, S), F32),
            pltpu.VMEM((S, D), BF16),
            pltpu.VMEM((D, S), BF16),
            pltpu.VMEM((3 * 128, 512), F32),
            pltpu.VMEM((M, D), BF16),
            pltpu.VMEM((D,), BF16),
            pltpu.SemaphoreType.DMA((46,)),
        ],
        compiler_params=pltpu.CompilerParams(vmem_limit_bytes=110 * 1024 * 1024),
    )(A_x.reshape(S, D).T, A_wqkv, A_wo, B_mem0.reshape(M, D),
      B_Wq.reshape(D // 2, 2 * HB, E), B_Wk.reshape(D // 2, 2 * HB, E), B_Wv.reshape(D // 2, 2 * HB, E),
      jnp.transpose(B_Wo, (0, 2, 1)).reshape(HB * D, E), gate_w)
    return outT.T.reshape(1, S, D)
```

```python
import functools
import math

import jax
import jax.numpy as jnp
from jax import lax
from jax.experimental import pallas as pl
from jax.experimental.pallas import tpu as pltpu

F32 = jnp.float32
BF16 = jnp.bfloat16
U32 = jnp.uint32
LOG2E = math.log2(math.e)
NEG = -1e9

NT = (((1,), (1,)), ((), ()))

DMA_ORDER = (("w", 0, 0), ("wo", 0), ("w", 0, 1), ("w", 1, 0), ("wo", 1), ("w", 1, 1), ("wo", 2), ("wo", 3),
             ("w", 2, 0), ("w", 2, 1))
FIN_T = (5, 7, 9, 11)
AOUT_T = 14
COMB_T = 2
LAG_E = (1, 3, 3)
LAG_O = (2, 4, 2)


def _dot(a, b):
    return jnp.dot(a, b, preferred_element_type=F32)


def _dot_nt(a, b):
    return lax.dot_general(a, b, NT, preferred_element_type=F32)


def _bf16_round(v):
    m, e = math.frexp(v)
    return math.ldexp(round(m * 256.0) / 256.0, e)


def _make_kernel(S, D, HA, W, HB, E, M, SEG):
    DHA = D // HA
    SLOT = 32
    DP = HA * SLOT
    QB = 128
    NQB = S // QB
    GPH = 128 // SLOT
    NG = HA // GPH
    PCH = 256
    NPC = S // PCH
    NP1 = 3
    NWO = 4
    HPW = HB // NWO
    HH = HB // 2
    assert SEG == 32 and M == 8 and W == 2 * QB and D % 16 == 0 and DHA < SLOT
    assert NPC - NP1 == 5 and NG == 4 and E == 256 and HB == 16
    cexp_a = _bf16_round(DHA ** -0.5) * LOG2E
    cexp_b = _bf16_round(E ** -0.5) * LOG2E

    def kernel(xaT_hbm, wqkv_hbm, wo_hbm, mem0_hbm, wq_hbm, wk_hbm, wv_hbm, woT_hbm, gate_hbm,
               outT_hbm,
               xaT, wqkv, wo, xb, wraw, wraw2, wpk, woTraw, wob, wTp, woTp, qT, kk, vT, gl, gaT, bb, outT, s0buf,
               mem0_ref, gate_ref, sems):
        cps = {}

        def start(name, src, dst, idx):
            cp = pltpu.make_async_copy(src, dst, sems.at[idx])
            cp.start()
            cps[name] = cp
        start("gate", gate_hbm, gate_ref, 32)
        start("mem0", mem0_hbm, mem0_ref, 33)
        start("wqkv", wqkv_hbm, wqkv, 0)

        def x_copy(c):
            col = pl.multiple_of(c * PCH, PCH)
            return pltpu.make_async_copy(xaT_hbm.at[:, pl.ds(col, PCH)], xaT.at[:, pl.ds(col, PCH)], sems.at[38 + c])
        for c in range(NPC):
            x_copy(c).start()
        start("wo", wo_hbm, wo, 2)

        def wc_copy(mi, t):
            wu = (wq_hbm, wk_hbm)[mi].bitcast(U32)
            dst = wraw2.at[mi * 2 + t].reshape(D // 2, HB, 128)
            return pltpu.make_async_copy(wu.at[:, :, t * 128:(t + 1) * 128], dst, sems.at[4 + mi * 2 + t])

        def wv_copy(t, par):
            wu = wv_hbm.bitcast(U32)
            dst = wraw.at[t * 2 + par].reshape(D // 2, HH, 128)
            return pltpu.make_async_copy(wu.at[:, par * HH:(par + 1) * HH, t * 128:(t + 1) * 128],
                                         dst, sems.at[8 + t * 2 + par])

        def w_copies(mi, t):
            return [wc_copy(mi, t)] if mi < 2 else [wv_copy(t, par) for par in range(2)]

        def w_wait(mi, t):
            for cp in w_copies(mi, t):
                cp.wait()

        def wo_copy(k):
            r0 = k * HPW * D
            return pltpu.make_async_copy(woT_hbm.at[pl.ds(r0, HPW * D)], woTraw.at[pl.ds(r0, HPW * D)],
                                         sems.at[34 + k])

        for item in DMA_ORDER:
            if item[0] == "w":
                for cp in w_copies(item[1], item[2]):
                    cp.start()
            else:
                wo_copy(item[1]).start()

        lane = lax.broadcasted_iota(jnp.int32, (W, DP), 1)
        kk[0:W, :] = jnp.where(lane % SLOT == DHA, NEG, 0.0).astype(BF16)
        vT[:, 0:W] = jnp.zeros((DP, W), BF16)
        gaT[:, 0:QB] = jnp.zeros((D, QB), F32)
        bb[0:QB, :] = jnp.zeros((QB, D), BF16)

        def respace(r, fill):
            n = r.shape[1]
            first = lax.broadcasted_iota(jnp.int32, (SLOT - DHA, n), 0) == 0
            pad = jnp.where(first, fill, 0.0).astype(r.dtype)
            parts = []
            for h in range(HA):
                parts += [r[h * DHA:(h + 1) * DHA], pad]
            return jnp.concatenate(parts, axis=0)

        cps["gate"].wait()
        cps["mem0"].wait()
        wTp[3 * D:3 * D + 16, :] = jnp.broadcast_to(gate_ref[...].reshape(1, D), (16, D))
        cps["wqkv"].wait()
        wTp[0:3 * D, :] = wqkv[...].T

        def proj(c):
            x_copy(c).wait()
            col = pl.multiple_of(c * PCH, PCH)
            xc = xaT[:, pl.ds(col, PCH)]
            qT[:, pl.ds(col, PCH)] = respace(_dot(wTp[0:D, :], xc) * cexp_a, 1.0).astype(BF16)
            kk[pl.ds(W + col, PCH), :] = respace(_dot(wTp[D:2 * D, :], xc), 0.0).astype(BF16).T
            r = _dot(wTp[2 * D:3 * D + 16, :], xc)
            vT[:, pl.ds(W + col, PCH)] = respace(r[0:D], 1.0).astype(BF16)
            gl[:, pl.ds(col, PCH)] = jax.nn.sigmoid(r[D:D + 8])
            xb[pl.ds(col, PCH), :] = xc.T

        def wob_head(h):
            wob[pl.ds(pl.multiple_of(h * E, E), E), :] = woTraw[pl.ds(pl.multiple_of(h * D, 16), D), :].T

        def relayout(xe, xo, mi, t, j):
            lo = (xe & U32(0xFFFF)) | (xo << 16)
            hi = (xe >> 16) | (xo & U32(0xFFFF0000))
            c0 = pl.multiple_of((2 * j) * 3 * E + mi * E + t * 128, 128)
            wpk[:, pl.ds(c0, 128)] = lo
            wpk[:, pl.ds(c0 + 3 * E, 128)] = hi

        def wc_unit(u):
            mt, j = u // HH, u % HH
            relayout(wraw2[mt, pl.ds(j, D // 2, stride=HB), :],
                     wraw2[mt, pl.ds(HH + j, D // 2, stride=HB), :], mt // 2, mt % 2, j)

        def wv_unit(u):
            t, j = u // HH, u % HH
            relayout(wraw[2 * t, pl.ds(j, D // 2, stride=HH), :],
                     wraw[2 * t + 1, pl.ds(j, D // 2, stride=HH), :], 2, t, j)

        def p1(c, carry):
            proj(c)
            return carry
        lax.fori_loop(0, NP1, p1, 0)
        cps["wo"].wait()
        woTp[...] = respace(wo[...].astype(F32), 0.0).T.astype(BF16)

        def piece_wait(n):
            w_wait(n // 2, n % 2)
            if n == 0:
                wo_copy(0).wait()
            elif n >= 2:
                wo_copy(n - 1).wait()

        def wob_piece(k):
            for n in range(HPW):
                wob_head(k * HPW + n)

        def p3(c, carry):
            for n in range(4):
                pl.when(c == NP1 + n)(functools.partial(piece_wait, n))
            proj(c)
            for k in range(HH):
                wc_unit((c - NP1) * HH + k)
            wob_piece(jnp.maximum(c - NP1 - 1, 0))
            return carry
        lax.fori_loop(NP1, NPC - 1, p3, 0)
        piece_wait(4)
        proj(NPC - 1)
        for k in range(HH):
            wv_unit(k)
        wob_piece(3)
        w_wait(2, 1)

        def p4(u, carry):
            wv_unit(HH + 2 * u)
            wv_unit(HH + 2 * u + 1)
            return carry
        lax.fori_loop(0, HH // 2, p4, 0)

        krow = lax.broadcasted_iota(jnp.int32, (QB, QB), 0)
        qcol = lax.broadcasted_iota(jnp.int32, (QB, QB), 1)
        upper = krow > qcol

        def a_scores(q0, g):
            kg = kk[pl.ds(q0, 3 * QB), g * 128:(g + 1) * 128]
            qg = qT[g * 128:(g + 1) * 128, pl.ds(q0, QB)]
            cols = []
            for j in range(GPH):
                parts = []
                if j > 0:
                    parts.append(jnp.zeros((j * SLOT, QB), BF16))
                parts.append(qg[j * SLOT:(j + 1) * SLOT])
                if j < GPH - 1:
                    parts.append(jnp.zeros((128 - (j + 1) * SLOT, QB), BF16))
                cols.append(jnp.concatenate(parts, axis=0))
            return _dot(kg, jnp.concatenate(cols, axis=1))

        def a_finish(q0, h, s):
            s0, s1, s2 = s[0:QB], s[QB:2 * QB], s[2 * QB:3 * QB]
            c = jnp.where(upper, s0, s2)
            m = jnp.maximum(jnp.max(c, axis=0, keepdims=True), jnp.max(s1, axis=0, keepdims=True))
            pc = jnp.exp2(c - m)
            p1_ = jnp.exp2(s1 - m)
            p = jnp.concatenate([jnp.where(upper, pc, 0.0), p1_, jnp.where(upper, 0.0, pc)], axis=0)
            vh = vT[h * SLOT:(h + 1) * SLOT, pl.ds(q0, 3 * QB)]
            o = _dot(vh, p.astype(BF16))
            return o * (1.0 / o[DHA:DHA + 1, :])

        def a_out(q0, oTs):
            oT = jnp.concatenate(oTs, axis=0)
            aT = _dot(woTp[...], oT.astype(BF16))
            aT = aT.astype(BF16).astype(F32)
            gaT[:, pl.ds(q0, QB)] = aT * gl[0:1, pl.ds(q0, QB)]

        rowE = lax.broadcasted_iota(jnp.int32, (32, 48), 0)
        colE = lax.broadcasted_iota(jnp.int32, (32, 48), 1)
        validE = (colE < M + SEG) & ((colE <= rowE) | (rowE < M))
        capE = jnp.where(validE, jnp.inf, NEG).astype(F32)
        rowO = lax.broadcasted_iota(jnp.int32, (48, 80), 0)
        colO = lax.broadcasted_iota(jnp.int32, (48, 80), 1)
        rtok = jnp.where(rowO < 32, rowO + 32, rowO - 8)
        ktok = jnp.where(colO < 48, colO - 8, colO - 16)
        k_m0 = colO < M
        k_m1 = (colO >= 48) & (colO < 48 + M)
        k_tok = jnp.logical_not(k_m0 | k_m1)
        r_mem = rowO < M
        r_seg1 = r_mem | (rtok >= SEG)
        validO = ((r_seg1 & (k_m1 | (k_tok & (ktok >= SEG) & ((ktok <= rtok) | r_mem)))) |
                  (jnp.logical_not(r_seg1) & (k_m0 | (k_tok & (ktok <= rtok)))))
        capO = jnp.where(validO, jnp.inf, NEG).astype(F32)

        def softmax_p(s, cap):
            s = jnp.minimum(s, cap)
            m = jnp.max(s, axis=-1, keepdims=True)
            e = jnp.exp2((s - m) * cexp_b)
            l = jnp.sum(e, axis=-1, keepdims=True)
            return e * (1.0 / l)

        def seg_step(hq, hin, prev, cap, hooks, ls, lp, nfill):
            qq = [None] * HB
            kv = [None] * HB
            p = [None] * HB
            v = [None] * HB
            o = [None] * HB

            def do_qkv(h):
                wq = pltpu.bitcast(wpk[:, h * 3 * E:h * 3 * E + E], BF16)
                wkv = pltpu.bitcast(wpk[:, h * 3 * E + E:(h + 1) * 3 * E], BF16)
                kv[h] = _dot(hin, wkv)
                qq[h] = _dot(hq, wq)

            def do_s(h):
                r = kv[h]
                if prev is None:
                    k, v[h] = r[:, :E], r[:, E:]
                else:
                    a = prev[h]
                    k = jnp.concatenate([a[:, :E], r[:, :E]], axis=0)
                    v[h] = jnp.concatenate([a[:, E:], r[:, E:]], axis=0)
                p[h] = softmax_p(_dot_nt(qq[h].astype(BF16), k.astype(BF16)), cap)

            def do_pv(h):
                o[h] = _dot(p[h].astype(BF16), v[h].astype(BF16))

            def do_wo(h, acc):
                r = _dot(o[h].astype(BF16), wob[h * E:(h + 1) * E, :])
                return r if acc is None else acc + r

            for t in range(HB):
                do_qkv(t)
                if t >= ls:
                    do_s(t - ls)
                if t >= lp:
                    do_pv(t - lp)
                for f in hooks.get(t, ()):
                    f()
            acc = None
            wo_next = 0
            for t in range(HB, HB + lp):
                for _ in range(nfill):
                    if wo_next < t - lp:
                        acc = do_wo(wo_next, acc)
                        wo_next += 1
                if t - ls < HB:
                    do_s(t - ls)
                do_pv(t - lp)
            for h in range(wo_next, HB):
                acc = do_wo(h, acc)
            for f in hooks.get("end", ()):
                f()
            return acc, kv

        def pair(base, mem, hooksE, hooksO):
            t8 = xb[pl.ds(base, 8), :].astype(F32)
            g0 = jnp.concatenate([mem, t8], axis=0).astype(BF16)
            g12 = xb[pl.ds(base + 8, 32), :]
            hA = jnp.concatenate([g0, g12], axis=0)
            resA, kvA = seg_step(hA[0:32], hA, None, capE, hooksE, *LAG_E)
            mem1 = resA[0:8].astype(BF16).astype(F32)
            t8b = xb[pl.ds(base + 40, 8), :].astype(F32)
            g0b = jnp.concatenate([mem1, t8b], axis=0).astype(BF16)
            g1b = xb[pl.ds(base + 48, 16), :]
            hB = jnp.concatenate([g0b, g1b], axis=0)
            hQ = jnp.concatenate([hB, hA[32:48]], axis=0)
            resB, _ = seg_step(hQ, hB, kvA, capO, hooksO, *LAG_O)
            mem2 = resB[0:8].astype(BF16).astype(F32)
            b64 = jnp.concatenate([resA[8:32], resB[32:48], resB[8:32]], axis=0)
            bb[pl.ds(base, 64), :] = b64.astype(BF16)
            return mem2

        def combine(c0):
            bT = bb[pl.ds(c0, QB), :].T.astype(F32)
            g = gl[0:1, pl.ds(c0, QB)]
            outT[:, pl.ds(c0, QB)] = (gaT[:, pl.ds(c0, QB)] + (1.0 - g) * bT).astype(BF16)

        def out_copy(b):
            c0 = pl.multiple_of(b * QB, QB)
            return pltpu.make_async_copy(outT.at[:, pl.ds(c0, QB)], outT_hbm.at[:, pl.ds(c0, QB)], sems.at[16 + b])

        def super_iter(j, mem):
            q0 = pl.multiple_of(j * QB, QB)
            sc = {}
            oTs = [None] * HA

            def keep_scores(g, r):
                for jj in range(GPH):
                    sc[g * GPH + jj] = r[:, jj * QB:(jj + 1) * QB]

            def finish(h):
                oTs[h] = a_finish(q0, h, sc[h])

            def next_scores():
                qn = pl.multiple_of(jnp.minimum(j + 1, NQB - 1) * QB, QB)
                s0buf[...] = a_scores(qn, 0)

            hk = []
            for g in range(NG):
                h_g = {}
                for jj in range(GPH):
                    h_g.setdefault(FIN_T[jj], []).append(functools.partial(finish, g * GPH + jj))
                if g + 1 < NG:
                    h_g["end"] = [lambda g=g: keep_scores(g + 1, a_scores(q0, g + 1))]
                else:
                    h_g.setdefault(AOUT_T, []).append(lambda: a_out(q0, oTs))
                    h_g["end"] = [next_scores]
                hk.append(h_g)
            hk[0].setdefault(COMB_T, []).append(
                lambda: combine(pl.multiple_of(jnp.maximum(j - 1, 0) * QB, QB)))

            keep_scores(0, s0buf[...])
            mem = pair(q0, mem, hk[0], hk[1])
            mem = pair(q0 + 64, mem, hk[2], hk[3])

            @pl.when(j > 0)
            def _():
                out_copy(j - 1).start()
            return mem

        s0buf[...] = a_scores(0, 0)
        lax.fori_loop(0, NQB, super_iter, mem0_ref[...].astype(F32))
        combine((NQB - 1) * QB)
        out_copy(NQB - 1).start()
        for b in range(NQB):
            out_copy(b).wait()

    return kernel


@functools.partial(jax.jit, static_argnames=("B_seg_len",))
def pallas_gated_mix__sliding_block__memory_aug_recurrent_mem_tr__prompt_kernel(
        A_x, A_wqkv, A_wo, B_x, B_mem0, B_Wq, B_Wk, B_Wv, B_Wo, B_seg_len, gate_w):
    del B_x
    Bn, S, D = A_x.shape
    assert Bn == 1
    HB, E = B_Wq.shape[1], B_Wq.shape[2]
    M = B_mem0.shape[1]
    HA, WIN = 16, 256
    kern = _make_kernel(S, D, HA, WIN, HB, E, M, B_seg_len)
    hbm_spec = pl.BlockSpec(memory_space=pltpu.MemorySpace.HBM)
    outT = pl.pallas_call(
        kern,
        out_shape=jax.ShapeDtypeStruct((D, S), BF16),
        in_specs=[hbm_spec] * 9,
        out_specs=hbm_spec,
        scratch_shapes=[
            pltpu.VMEM((D, S), BF16),
            pltpu.VMEM((D, 3 * D), BF16),
            pltpu.VMEM((D, D), BF16),
            pltpu.VMEM((S, D), BF16),
            pltpu.VMEM((4, D * HB // 4, 128), U32),
            pltpu.VMEM((4, D * HB // 2, 128), U32),
            pltpu.VMEM((D // 2, 3 * HB * E), U32),
            pltpu.VMEM((HB * D, E), BF16),
            pltpu.VMEM((HB * E, D), BF16),
            pltpu.VMEM((3 * D + 16, D), BF16),
            pltpu.VMEM((D, 512), BF16),
            pltpu.VMEM((512, S), BF16),
            pltpu.VMEM((WIN + S, 512), BF16),
            pltpu.VMEM((512, WIN + S), BF16),
            pltpu.VMEM((8, S), F32),
            pltpu.VMEM((D, S), F32),
            pltpu.VMEM((S, D), BF16),
            pltpu.VMEM((D, S), BF16),
            pltpu.VMEM((3 * 128, 512), F32),
            pltpu.VMEM((M, D), BF16),
            pltpu.VMEM((D,), BF16),
            pltpu.SemaphoreType.DMA((46,)),
        ],
        compiler_params=pltpu.CompilerParams(vmem_limit_bytes=110 * 1024 * 1024),
    )(A_x.reshape(S, D).T, A_wqkv, A_wo, B_mem0.reshape(M, D),
      B_Wq.reshape(D // 2, 2 * HB, E), B_Wk.reshape(D // 2, 2 * HB, E), B_Wv.reshape(D // 2, 2 * HB, E),
      jnp.transpose(B_Wo, (0, 2, 1)).reshape(HB * D, E), gate_w)
    return outT.T.reshape(1, S, D)
```

```python
import functools
import math

import jax
import jax.numpy as jnp
from jax import lax
from jax.experimental import pallas as pl
from jax.experimental.pallas import tpu as pltpu

F32 = jnp.float32
BF16 = jnp.bfloat16
U32 = jnp.uint32
LOG2E = math.log2(math.e)
NEG = -1e9

NT = (((1,), (1,)), ((), ()))

DMA_ORDER = (("w", 0, 0), ("wo", 0), ("w", 0, 1), ("w", 1, 0), ("wo", 1), ("w", 1, 1), ("wo", 2), ("wo", 3),
             ("w", 2, 0), ("w", 2, 1))
FIN_T = (5, 7, 9, 11)
AOUT_T = 14
COMB_T = 2
LAG_E = (1, 3, 3)
LAG_O = (2, 4, 2)


def _dot(a, b):
    return jnp.dot(a, b, preferred_element_type=F32)


def _dot_nt(a, b):
    return lax.dot_general(a, b, NT, preferred_element_type=F32)


def _bf16_round(v):
    m, e = math.frexp(v)
    return math.ldexp(round(m * 256.0) / 256.0, e)


def _make_kernel(S, D, HA, W, HB, E, M, SEG):
    DHA = D // HA
    SLOT = 32
    DP = HA * SLOT
    QB = 128
    NQB = S // QB
    GPH = 128 // SLOT
    NG = HA // GPH
    PCH = 256
    NPC = S // PCH
    NP1 = 3
    NWO = 4
    HPW = HB // NWO
    HH = HB // 2
    assert SEG == 32 and M == 8 and W == 2 * QB and D % 16 == 0 and DHA < SLOT
    assert NPC - NP1 == 5 and NG == 4 and E == 256 and HB == 16
    cexp_a = _bf16_round(DHA ** -0.5) * LOG2E
    cexp_b = _bf16_round(E ** -0.5) * LOG2E

    def kernel(xaT_hbm, wqkv_hbm, wo_hbm, mem0_hbm, wq_hbm, wk_hbm, wv_hbm, woT_hbm, gate_hbm,
               outT_hbm,
               xaT, wqkv, wo, xb, wraw, wraw2, wpk, woTraw, wob, wTp, woTp, qT, kk, vT, gl, gaT, bb, outT, s0buf,
               mem0_ref, gate_ref, sems):
        cps = {}

        def start(name, src, dst, idx):
            cp = pltpu.make_async_copy(src, dst, sems.at[idx])
            cp.start()
            cps[name] = cp
        start("gate", gate_hbm, gate_ref, 32)
        start("mem0", mem0_hbm, mem0_ref, 33)
        start("wqkv", wqkv_hbm, wqkv, 0)

        def x_copy(c):
            col = pl.multiple_of(c * PCH, PCH)
            return pltpu.make_async_copy(xaT_hbm.at[:, pl.ds(col, PCH)], xaT.at[:, pl.ds(col, PCH)], sems.at[38 + c])
        for c in range(NPC):
            x_copy(c).start()
        start("wo", wo_hbm, wo, 2)

        def wc_copy(mi, t):
            wu = (wq_hbm, wk_hbm)[mi].bitcast(U32)
            dst = wraw2.at[mi * 2 + t].reshape(D // 2, HB, 128)
            return pltpu.make_async_copy(wu.at[:, :, t * 128:(t + 1) * 128], dst, sems.at[4 + mi * 2 + t])

        def wv_copy(t, par):
            wu = wv_hbm.bitcast(U32)
            dst = wraw.at[t * 2 + par].reshape(D // 2, HH, 128)
            return pltpu.make_async_copy(wu.at[:, par * HH:(par + 1) * HH, t * 128:(t + 1) * 128],
                                         dst, sems.at[8 + t * 2 + par])

        def w_copies(mi, t):
            return [wc_copy(mi, t)] if mi < 2 else [wv_copy(t, par) for par in range(2)]

        def w_wait(mi, t):
            for cp in w_copies(mi, t):
                cp.wait()

        def wo_copy(k):
            r0 = k * HPW * D
            return pltpu.make_async_copy(woT_hbm.at[pl.ds(r0, HPW * D)], woTraw.at[pl.ds(r0, HPW * D)],
                                         sems.at[34 + k])

        for item in DMA_ORDER:
            if item[0] == "w":
                for cp in w_copies(item[1], item[2]):
                    cp.start()
            else:
                wo_copy(item[1]).start()

        lane = lax.broadcasted_iota(jnp.int32, (W, DP), 1)
        kk[0:W, :] = jnp.where(lane % SLOT == DHA, NEG, 0.0).astype(BF16)
        vT[:, 0:W] = jnp.zeros((DP, W), BF16)
        gaT[:, 0:QB] = jnp.zeros((D, QB), F32)
        bb[0:QB, :] = jnp.zeros((QB, D), BF16)

        def respace(r, fill):
            n = r.shape[1]
            first = lax.broadcasted_iota(jnp.int32, (SLOT - DHA, n), 0) == 0
            pad = jnp.where(first, fill, 0.0).astype(r.dtype)
            parts = []
            for h in range(HA):
                parts += [r[h * DHA:(h + 1) * DHA], pad]
            return jnp.concatenate(parts, axis=0)

        cps["gate"].wait()
        cps["mem0"].wait()
        wTp[3 * D:3 * D + 16, :] = jnp.broadcast_to(gate_ref[...].reshape(1, D), (16, D))
        cps["wqkv"].wait()
        wTp[0:3 * D, :] = wqkv[...].T

        def proj(c):
            x_copy(c).wait()
            col = pl.multiple_of(c * PCH, PCH)
            xc = xaT[:, pl.ds(col, PCH)]
            qT[:, pl.ds(col, PCH)] = respace(_dot(wTp[0:D, :], xc) * cexp_a, 1.0).astype(BF16)
            kk[pl.ds(W + col, PCH), :] = respace(_dot(wTp[D:2 * D, :], xc), 0.0).astype(BF16).T
            r = _dot(wTp[2 * D:3 * D + 16, :], xc)
            vT[:, pl.ds(W + col, PCH)] = respace(r[0:D], 1.0).astype(BF16)
            gl[:, pl.ds(col, PCH)] = jax.nn.sigmoid(r[D:D + 8])
            xb[pl.ds(col, PCH), :] = xc.T

        def wob_head(h):
            wob[pl.ds(pl.multiple_of(h * E, E), E), :] = woTraw[pl.ds(pl.multiple_of(h * D, 16), D), :].T

        def relayout(xe, xo, mi, t, j):
            lo = (xe & U32(0xFFFF)) | (xo << 16)
            hi = (xe >> 16) | (xo & U32(0xFFFF0000))
            c0 = pl.multiple_of((2 * j) * 3 * E + mi * E + t * 128, 128)
            wpk[:, pl.ds(c0, 128)] = lo
            wpk[:, pl.ds(c0 + 3 * E, 128)] = hi

        def wc_unit(u):
            mt, j = u // HH, u % HH
            relayout(wraw2[mt, pl.ds(j, D // 2, stride=HB), :],
                     wraw2[mt, pl.ds(HH + j, D // 2, stride=HB), :], mt // 2, mt % 2, j)

        def wv_unit(u):
            t, j = u // HH, u % HH
            relayout(wraw[2 * t, pl.ds(j, D // 2, stride=HH), :],
                     wraw[2 * t + 1, pl.ds(j, D // 2, stride=HH), :], 2, t, j)

        def p1(c, carry):
            proj(c)
            return carry
        lax.fori_loop(0, NP1, p1, 0)
        cps["wo"].wait()
        woTp[...] = respace(wo[...].astype(F32), 0.0).T.astype(BF16)

        def piece_wait(n):
            w_wait(n // 2, n % 2)
            if n == 0:
                wo_copy(0).wait()
            elif n >= 2:
                wo_copy(n - 1).wait()

        def wob_piece(k):
            for n in range(HPW):
                wob_head(k * HPW + n)

        def p3(c, carry):
            for n in range(4):
                pl.when(c == NP1 + n)(functools.partial(piece_wait, n))
            proj(c)
            for k in range(HH):
                wc_unit((c - NP1) * HH + k)
            wob_piece(jnp.maximum(c - NP1 - 1, 0))
            return carry
        lax.fori_loop(NP1, NPC - 1, p3, 0)
        piece_wait(4)
        proj(NPC - 1)
        for k in range(HH):
            wv_unit(k)
        wob_piece(3)
        w_wait(2, 1)

        def p4(u, carry):
            wv_unit(HH + 2 * u)
            wv_unit(HH + 2 * u + 1)
            return carry
        lax.fori_loop(0, HH // 2, p4, 0)

        krow = lax.broadcasted_iota(jnp.int32, (QB, QB), 0)
        qcol = lax.broadcasted_iota(jnp.int32, (QB, QB), 1)
        upper = krow > qcol

        def a_scores(q0, g):
            kg = kk[pl.ds(q0, 3 * QB), g * 128:(g + 1) * 128]
            qg = qT[g * 128:(g + 1) * 128, pl.ds(q0, QB)]
            cols = []
            for j in range(GPH):
                parts = []
                if j > 0:
                    parts.append(jnp.zeros((j * SLOT, QB), BF16))
                parts.append(qg[j * SLOT:(j + 1) * SLOT])
                if j < GPH - 1:
                    parts.append(jnp.zeros((128 - (j + 1) * SLOT, QB), BF16))
                cols.append(jnp.concatenate(parts, axis=0))
            return _dot(kg, jnp.concatenate(cols, axis=1))

        def a_finish(q0, h, s):
            s0, s1, s2 = s[0:QB], s[QB:2 * QB], s[2 * QB:3 * QB]
            c = jnp.where(upper, s0, s2)
            m = jnp.maximum(jnp.max(c, axis=0, keepdims=True), jnp.max(s1, axis=0, keepdims=True))
            pc = jnp.exp2(c - m)
            p1_ = jnp.exp2(s1 - m)
            p = jnp.concatenate([jnp.where(upper, pc, 0.0), p1_, jnp.where(upper, 0.0, pc)], axis=0)
            vh = vT[h * SLOT:(h + 1) * SLOT, pl.ds(q0, 3 * QB)]
            o = _dot(vh, p.astype(BF16))
            return o * (1.0 / o[DHA:DHA + 1, :])

        def a_out(q0, oTs):
            oT = jnp.concatenate(oTs, axis=0)
            aT = _dot(woTp[...], oT.astype(BF16))
            aT = aT.astype(BF16).astype(F32)
            gaT[:, pl.ds(q0, QB)] = aT * gl[0:1, pl.ds(q0, QB)]

        rowE = lax.broadcasted_iota(jnp.int32, (32, 48), 0)
        colE = lax.broadcasted_iota(jnp.int32, (32, 48), 1)
        validE = (colE < M + SEG) & ((colE <= rowE) | (rowE < M))
        capE = jnp.where(validE, jnp.inf, NEG).astype(F32)
        rowO = lax.broadcasted_iota(jnp.int32, (48, 80), 0)
        colO = lax.broadcasted_iota(jnp.int32, (48, 80), 1)
        rtok = jnp.where(rowO < 32, rowO + 32, rowO - 8)
        ktok = jnp.where(colO < 48, colO - 8, colO - 16)
        k_m0 = colO < M
        k_m1 = (colO >= 48) & (colO < 48 + M)
        k_tok = jnp.logical_not(k_m0 | k_m1)
        r_mem = rowO < M
        r_seg1 = r_mem | (rtok >= SEG)
        validO = ((r_seg1 & (k_m1 | (k_tok & (ktok >= SEG) & ((ktok <= rtok) | r_mem)))) |
                  (jnp.logical_not(r_seg1) & (k_m0 | (k_tok & (ktok <= rtok)))))
        capO = jnp.where(validO, jnp.inf, NEG).astype(F32)

        def softmax_p(s, cap):
            s = jnp.minimum(s, cap)
            m = jnp.max(s, axis=-1, keepdims=True)
            e = jnp.exp2((s - m) * cexp_b)
            l = jnp.sum(e, axis=-1, keepdims=True)
            return e * (1.0 / l)

        def seg_step(hq, hin, prev, cap, hooks, ls, lp, nfill):
            qq = [None] * HB
            kv = [None] * HB
            p = [None] * HB
            v = [None] * HB
            o = [None] * HB

            def do_qkv(h):
                wq = pltpu.bitcast(wpk[:, h * 3 * E:h * 3 * E + E], BF16)
                wkv = pltpu.bitcast(wpk[:, h * 3 * E + E:(h + 1) * 3 * E], BF16)
                kv[h] = _dot(hin, wkv)
                qq[h] = _dot(hq, wq)

            def do_s(h):
                r = kv[h]
                if prev is None:
                    k, v[h] = r[:, :E], r[:, E:]
                else:
                    a = prev[h]
                    k = jnp.concatenate([a[:, :E], r[:, :E]], axis=0)
                    v[h] = jnp.concatenate([a[:, E:], r[:, E:]], axis=0)
                p[h] = softmax_p(_dot_nt(qq[h].astype(BF16), k.astype(BF16)), cap)

            def do_pv(h):
                o[h] = _dot(p[h].astype(BF16), v[h].astype(BF16))

            def do_wo(h, acc):
                r = _dot(o[h].astype(BF16), wob[h * E:(h + 1) * E, :])
                return r if acc is None else acc + r

            for t in range(HB):
                do_qkv(t)
                if t >= ls:
                    do_s(t - ls)
                if t >= lp:
                    do_pv(t - lp)
                for f in hooks.get(t, ()):
                    f()
            acc = None
            wo_next = 0
            for t in range(HB, HB + lp):
                for _ in range(nfill):
                    if wo_next < t - lp:
                        acc = do_wo(wo_next, acc)
                        wo_next += 1
                if t - ls < HB:
                    do_s(t - ls)
                do_pv(t - lp)
            for h in range(wo_next, HB):
                acc = do_wo(h, acc)
            for f in hooks.get("end", ()):
                f()
            return acc, kv

        def pair(base, mem, hooksE, hooksO):
            t8 = xb[pl.ds(base, 8), :].astype(F32)
            g0 = jnp.concatenate([mem, t8], axis=0).astype(BF16)
            g12 = xb[pl.ds(base + 8, 32), :]
            hA = jnp.concatenate([g0, g12], axis=0)
            resA, kvA = seg_step(hA[0:32], hA, None, capE, hooksE, *LAG_E)
            mem1 = resA[0:8].astype(BF16).astype(F32)
            t8b = xb[pl.ds(base + 40, 8), :].astype(F32)
            g0b = jnp.concatenate([mem1, t8b], axis=0).astype(BF16)
            g1b = xb[pl.ds(base + 48, 16), :]
            hB = jnp.concatenate([g0b, g1b], axis=0)
            hQ = jnp.concatenate([hB, hA[32:48]], axis=0)
            resB, _ = seg_step(hQ, hB, kvA, capO, hooksO, *LAG_O)
            mem2 = resB[0:8].astype(BF16).astype(F32)
            b64 = jnp.concatenate([resA[8:32], resB[32:48], resB[8:32]], axis=0)
            bb[pl.ds(base, 64), :] = b64.astype(BF16)
            return mem2

        def combine(c0):
            bT = bb[pl.ds(c0, QB), :].T.astype(F32)
            g = gl[0:1, pl.ds(c0, QB)]
            outT[:, pl.ds(c0, QB)] = (gaT[:, pl.ds(c0, QB)] + (1.0 - g) * bT).astype(BF16)

        def out_copy(b):
            c0 = pl.multiple_of(b * QB, QB)
            return pltpu.make_async_copy(outT.at[:, pl.ds(c0, QB)], outT_hbm.at[:, pl.ds(c0, QB)], sems.at[16 + b])

        def super_iter(j, mem):
            q0 = pl.multiple_of(j * QB, QB)
            sc = {}
            oTs = [None] * HA

            def keep_scores(g, r):
                for jj in range(GPH):
                    sc[g * GPH + jj] = r[:, jj * QB:(jj + 1) * QB]

            def finish(h):
                oTs[h] = a_finish(q0, h, sc[h])

            def next_scores():
                qn = pl.multiple_of(jnp.minimum(j + 1, NQB - 1) * QB, QB)
                s0buf[...] = a_scores(qn, 0)

            hk = []
            for g in range(NG):
                h_g = {}
                for jj in range(GPH):
                    h_g.setdefault(FIN_T[jj], []).append(functools.partial(finish, g * GPH + jj))
                if g + 1 < NG:
                    h_g["end"] = [lambda g=g: keep_scores(g + 1, a_scores(q0, g + 1))]
                else:
                    h_g.setdefault(AOUT_T, []).append(lambda: a_out(q0, oTs))
                    h_g["end"] = [next_scores]
                hk.append(h_g)
            hk[0].setdefault(COMB_T, []).append(
                lambda: combine(pl.multiple_of(jnp.maximum(j - 1, 0) * QB, QB)))

            keep_scores(0, s0buf[...])
            mem = pair(q0, mem, hk[0], hk[1])
            mem = pair(q0 + 64, mem, hk[2], hk[3])
            return mem

        def double_iter(i, mem):
            mem = super_iter(2 * i, mem)
            mem = super_iter(2 * i + 1, mem)
            out_copy(2 * i).start()

            @pl.when(i > 0)
            def _():
                out_copy(2 * i - 1).start()
            return mem

        s0buf[...] = a_scores(0, 0)
        lax.fori_loop(0, NQB // 2, double_iter, mem0_ref[...].astype(F32))
        combine((NQB - 1) * QB)
        out_copy(NQB - 1).start()
        for b in range(NQB):
            out_copy(b).wait()

    return kernel


@functools.partial(jax.jit, static_argnames=("B_seg_len",))
def pallas_gated_mix__sliding_block__memory_aug_recurrent_mem_tr__prompt_kernel(
        A_x, A_wqkv, A_wo, B_x, B_mem0, B_Wq, B_Wk, B_Wv, B_Wo, B_seg_len, gate_w):
    del B_x
    Bn, S, D = A_x.shape
    assert Bn == 1
    HB, E = B_Wq.shape[1], B_Wq.shape[2]
    M = B_mem0.shape[1]
    HA, WIN = 16, 256
    kern = _make_kernel(S, D, HA, WIN, HB, E, M, B_seg_len)
    hbm_spec = pl.BlockSpec(memory_space=pltpu.MemorySpace.HBM)
    outT = pl.pallas_call(
        kern,
        out_shape=jax.ShapeDtypeStruct((D, S), BF16),
        in_specs=[hbm_spec] * 9,
        out_specs=hbm_spec,
        scratch_shapes=[
            pltpu.VMEM((D, S), BF16),
            pltpu.VMEM((D, 3 * D), BF16),
            pltpu.VMEM((D, D), BF16),
            pltpu.VMEM((S, D), BF16),
            pltpu.VMEM((4, D * HB // 4, 128), U32),
            pltpu.VMEM((4, D * HB // 2, 128), U32),
            pltpu.VMEM((D // 2, 3 * HB * E), U32),
            pltpu.VMEM((HB * D, E), BF16),
            pltpu.VMEM((HB * E, D), BF16),
            pltpu.VMEM((3 * D + 16, D), BF16),
            pltpu.VMEM((D, 512), BF16),
            pltpu.VMEM((512, S), BF16),
            pltpu.VMEM((WIN + S, 512), BF16),
            pltpu.VMEM((512, WIN + S), BF16),
            pltpu.VMEM((8, S), F32),
            pltpu.VMEM((D, S), F32),
            pltpu.VMEM((S, D), BF16),
            pltpu.VMEM((D, S), BF16),
            pltpu.VMEM((3 * 128, 512), F32),
            pltpu.VMEM((M, D), BF16),
            pltpu.VMEM((D,), BF16),
            pltpu.SemaphoreType.DMA((46,)),
        ],
        compiler_params=pltpu.CompilerParams(vmem_limit_bytes=110 * 1024 * 1024),
    )(A_x.reshape(S, D).T, A_wqkv, A_wo, B_mem0.reshape(M, D),
      B_Wq.reshape(D // 2, 2 * HB, E), B_Wk.reshape(D // 2, 2 * HB, E), B_Wv.reshape(D // 2, 2 * HB, E),
      jnp.transpose(B_Wo, (0, 2, 1)).reshape(HB * D, E), gate_w)
    return outT.T.reshape(1, S, D)
```

```python
import functools
import math

import jax
import jax.numpy as jnp
from jax import lax
from jax.experimental import pallas as pl
from jax.experimental.pallas import tpu as pltpu

F32 = jnp.float32
BF16 = jnp.bfloat16
U32 = jnp.uint32
LOG2E = math.log2(math.e)
NEG = -1e9

NT = (((1,), (1,)), ((), ()))

DMA_ORDER = (("w", 0, 0), ("wo", 0), ("w", 0, 1), ("w", 1, 0), ("wo", 1), ("w", 1, 1), ("wo", 2), ("wo", 3),
             ("w", 2, 0), ("w", 2, 1))
FIN_T = (5, 7, 9, 11)
AOUT_T = 14
COMB_T = 2
LAG_E = (1, 3, 3)
LAG_O = (2, 4, 2)


def _dot(a, b):
    return jnp.dot(a, b, preferred_element_type=F32)


def _dot_nt(a, b):
    return lax.dot_general(a, b, NT, preferred_element_type=F32)


def _bf16_round(v):
    m, e = math.frexp(v)
    return math.ldexp(round(m * 256.0) / 256.0, e)


def _make_kernel(S, D, HA, W, HB, E, M, SEG):
    DHA = D // HA
    SLOT = 32
    DP = HA * SLOT
    QB = 128
    NQB = S // QB
    GPH = 128 // SLOT
    NG = HA // GPH
    PCH = 256
    NPC = S // PCH
    NP1 = 3
    NWO = 4
    HPW = HB // NWO
    HH = HB // 2
    assert SEG == 32 and M == 8 and W == 2 * QB and D % 16 == 0 and DHA < SLOT
    assert NPC - NP1 == 5 and NG == 4 and E == 256 and HB == 16
    cexp_a = _bf16_round(DHA ** -0.5) * LOG2E
    cexp_b = _bf16_round(E ** -0.5) * LOG2E

    def kernel(xaT_hbm, wqkv_hbm, wo_hbm, mem0_hbm, wq_hbm, wk_hbm, wv_hbm, woT_hbm, gate_hbm,
               outT_hbm,
               xaT, wqkv, wo, xb, wraw, wraw2, wpk, woTraw, wob, wTp, woTp, qT, kk, vT, gl, gaT, bb, outT, s0buf,
               mem0_ref, gate_ref, sems):
        cps = {}

        def start(name, src, dst, idx):
            cp = pltpu.make_async_copy(src, dst, sems.at[idx])
            cp.start()
            cps[name] = cp
        start("gate", gate_hbm, gate_ref, 32)
        start("mem0", mem0_hbm, mem0_ref, 33)
        start("wqkv", wqkv_hbm, wqkv, 0)

        def x_copy(c):
            col = pl.multiple_of(c * PCH, PCH)
            return pltpu.make_async_copy(xaT_hbm.at[:, pl.ds(col, PCH)], xaT.at[:, pl.ds(col, PCH)], sems.at[38 + c])
        for c in range(NPC):
            x_copy(c).start()
        start("wo", wo_hbm, wo, 2)

        def wc_copy(mi, t):
            wu = (wq_hbm, wk_hbm)[mi].bitcast(U32)
            dst = wraw2.at[mi * 2 + t, pl.ds(0, D // 2 * HB)].reshape(D // 2, HB, 128)
            return pltpu.make_async_copy(wu.at[:, :, t * 128:(t + 1) * 128], dst, sems.at[4 + mi * 2 + t])

        def wv_copy(t, par):
            wu = wv_hbm.bitcast(U32)
            dst = wraw.at[t * 2 + par, pl.ds(0, D // 2 * HH)].reshape(D // 2, HH, 128)
            return pltpu.make_async_copy(wu.at[:, par * HH:(par + 1) * HH, t * 128:(t + 1) * 128],
                                         dst, sems.at[8 + t * 2 + par])

        def w_copies(mi, t):
            return [wc_copy(mi, t)] if mi < 2 else [wv_copy(t, par) for par in range(2)]

        def w_wait(mi, t):
            for cp in w_copies(mi, t):
                cp.wait()

        def wo_copy(k):
            r0 = k * HPW * D
            return pltpu.make_async_copy(woT_hbm.at[pl.ds(r0, HPW * D)], woTraw.at[pl.ds(r0, HPW * D)],
                                         sems.at[34 + k])

        for item in DMA_ORDER:
            if item[0] == "w":
                for cp in w_copies(item[1], item[2]):
                    cp.start()
            else:
                wo_copy(item[1]).start()

        lane = lax.broadcasted_iota(jnp.int32, (W, DP), 1)
        kk[0:W, :] = jnp.where(lane % SLOT == DHA, NEG, 0.0).astype(BF16)
        vT[:, 0:W] = jnp.zeros((DP, W), BF16)
        gaT[:, 0:QB] = jnp.zeros((D, QB), F32)
        bb[0:QB, :] = jnp.zeros((QB, D), BF16)

        def respace(r, fill):
            n = r.shape[1]
            first = lax.broadcasted_iota(jnp.int32, (SLOT - DHA, n), 0) == 0
            pad = jnp.where(first, fill, 0.0).astype(r.dtype)
            parts = []
            for h in range(HA):
                parts += [r[h * DHA:(h + 1) * DHA], pad]
            return jnp.concatenate(parts, axis=0)

        cps["gate"].wait()
        cps["mem0"].wait()
        wTp[3 * D:3 * D + 16, :] = jnp.broadcast_to(gate_ref[...].reshape(1, D), (16, D))
        cps["wqkv"].wait()
        wTp[0:3 * D, :] = wqkv[...].T

        def proj(c):
            x_copy(c).wait()
            col = pl.multiple_of(c * PCH, PCH)
            xc = xaT[:, pl.ds(col, PCH)]
            qT[:, pl.ds(col, PCH)] = respace(_dot(wTp[0:D, :], xc) * cexp_a, 1.0).astype(BF16)
            kk[pl.ds(W + col, PCH), :] = respace(_dot(wTp[D:2 * D, :], xc), 0.0).astype(BF16).T
            r = _dot(wTp[2 * D:3 * D + 16, :], xc)
            vT[:, pl.ds(W + col, PCH)] = respace(r[0:D], 1.0).astype(BF16)
            gl[:, pl.ds(col, PCH)] = jax.nn.sigmoid(r[D:D + 8])
            xb[pl.ds(col, PCH), :] = xc.T

        def wob_head(h):
            wob[pl.ds(pl.multiple_of(h * E, E), E), :] = woTraw[pl.ds(pl.multiple_of(h * D, 16), D), :].T

        def relayout(xe, xo, mi, t, j):
            lo = (xe & U32(0xFFFF)) | (xo << 16)
            hi = (xe >> 16) | (xo & U32(0xFFFF0000))
            c0 = pl.multiple_of((2 * j) * 3 * E + mi * E + t * 128, 128)
            wpk[:, pl.ds(c0, 128)] = lo
            wpk[:, pl.ds(c0 + 3 * E, 128)] = hi

        def wc_unit(u):
            mt, j = u // HH, u % HH
            relayout(wraw2[mt, pl.ds(j, D // 2, stride=HB), :],
                     wraw2[mt, pl.ds(HH + j, D // 2, stride=HB), :], mt // 2, mt % 2, j)

        def wv_unit(u):
            t, j = u // HH, u % HH
            relayout(wraw[2 * t, pl.ds(j, D // 2, stride=HH), :],
                     wraw[2 * t + 1, pl.ds(j, D // 2, stride=HH), :], 2, t, j)

        def p1(c, carry):
            proj(c)
            return carry
        lax.fori_loop(0, NP1, p1, 0)
        cps["wo"].wait()
        woTp[...] = respace(wo[...].astype(F32), 0.0).T.astype(BF16)

        def piece_wait(n):
            w_wait(n // 2, n % 2)
            if n == 0:
                wo_copy(0).wait()
            elif n >= 2:
                wo_copy(n - 1).wait()

        def wob_piece(k):
            for n in range(HPW):
                wob_head(k * HPW + n)

        def p3(c, carry):
            for n in range(4):
                pl.when(c == NP1 + n)(functools.partial(piece_wait, n))
            proj(c)
            for k in range(HH):
                wc_unit((c - NP1) * HH + k)
            wob_piece(jnp.maximum(c - NP1 - 1, 0))
            return carry
        lax.fori_loop(NP1, NPC - 1, p3, 0)
        piece_wait(4)
        proj(NPC - 1)
        for k in range(HH):
            wv_unit(k)
        wob_piece(3)
        w_wait(2, 1)

        def p4(u, carry):
            wv_unit(HH + 2 * u)
            wv_unit(HH + 2 * u + 1)
            return carry
        lax.fori_loop(0, HH // 2, p4, 0)

        krow = lax.broadcasted_iota(jnp.int32, (QB, QB), 0)
        qcol = lax.broadcasted_iota(jnp.int32, (QB, QB), 1)
        upper = krow > qcol

        def a_scores(q0, g):
            kg = kk[pl.ds(q0, 3 * QB), g * 128:(g + 1) * 128]
            qg = qT[g * 128:(g + 1) * 128, pl.ds(q0, QB)]
            cols = []
            for j in range(GPH):
                parts = []
                if j > 0:
                    parts.append(jnp.zeros((j * SLOT, QB), BF16))
                parts.append(qg[j * SLOT:(j + 1) * SLOT])
                if j < GPH - 1:
                    parts.append(jnp.zeros((128 - (j + 1) * SLOT, QB), BF16))
                cols.append(jnp.concatenate(parts, axis=0))
            return _dot(kg, jnp.concatenate(cols, axis=1))

        def a_finish(q0, h, s):
            s0, s1, s2 = s[0:QB], s[QB:2 * QB], s[2 * QB:3 * QB]
            c = jnp.where(upper, s0, s2)
            m = jnp.maximum(jnp.max(c, axis=0, keepdims=True), jnp.max(s1, axis=0, keepdims=True))
            pc = jnp.exp2(c - m)
            p1_ = jnp.exp2(s1 - m)
            p = jnp.concatenate([jnp.where(upper, pc, 0.0), p1_, jnp.where(upper, 0.0, pc)], axis=0)
            vh = vT[h * SLOT:(h + 1) * SLOT, pl.ds(q0, 3 * QB)]
            o = _dot(vh, p.astype(BF16))
            return o * (1.0 / o[DHA:DHA + 1, :])

        def a_out(q0, oTs):
            oT = jnp.concatenate(oTs, axis=0)
            aT = _dot(woTp[...], oT.astype(BF16))
            aT = aT.astype(BF16).astype(F32)
            gaT[:, pl.ds(q0, QB)] = aT * gl[0:1, pl.ds(q0, QB)]

        rowE = lax.broadcasted_iota(jnp.int32, (32, 48), 0)
        colE = lax.broadcasted_iota(jnp.int32, (32, 48), 1)
        validE = (colE < M + SEG) & ((colE <= rowE) | (rowE < M))
        capE = jnp.where(validE, jnp.inf, NEG).astype(F32)
        rowO = lax.broadcasted_iota(jnp.int32, (48, 80), 0)
        colO = lax.broadcasted_iota(jnp.int32, (48, 80), 1)
        rtok = jnp.where(rowO < 32, rowO + 32, rowO - 8)
        ktok = jnp.where(colO < 48, colO - 8, colO - 16)
        k_m0 = colO < M
        k_m1 = (colO >= 48) & (colO < 48 + M)
        k_tok = jnp.logical_not(k_m0 | k_m1)
        r_mem = rowO < M
        r_seg1 = r_mem | (rtok >= SEG)
        validO = ((r_seg1 & (k_m1 | (k_tok & (ktok >= SEG) & ((ktok <= rtok) | r_mem)))) |
                  (jnp.logical_not(r_seg1) & (k_m0 | (k_tok & (ktok <= rtok)))))
        capO = jnp.where(validO, jnp.inf, NEG).astype(F32)

        def softmax_p(s, cap):
            s = jnp.minimum(s, cap)
            m = jnp.max(s, axis=-1, keepdims=True)
            e = jnp.exp2((s - m) * cexp_b)
            l = jnp.sum(e, axis=-1, keepdims=True)
            return e * (1.0 / l)

        def seg_step(hq, hin, prev, cap, hooks, ls, lp, nfill):
            qq = [None] * HB
            kv = [None] * HB
            p = [None] * HB
            v = [None] * HB
            o = [None] * HB

            def do_qkv(h):
                wq = pltpu.bitcast(wpk[:, h * 3 * E:h * 3 * E + E], BF16)
                wkv = pltpu.bitcast(wpk[:, h * 3 * E + E:(h + 1) * 3 * E], BF16)
                kv[h] = _dot(hin, wkv)
                qq[h] = _dot(hq, wq)

            def do_s(h):
                r = kv[h]
                if prev is None:
                    k, v[h] = r[:, :E], r[:, E:]
                else:
                    a = prev[h]
                    k = jnp.concatenate([a[:, :E], r[:, :E]], axis=0)
                    v[h] = jnp.concatenate([a[:, E:], r[:, E:]], axis=0)
                p[h] = softmax_p(_dot_nt(qq[h].astype(BF16), k.astype(BF16)), cap)

            def do_pv(h):
                o[h] = _dot(p[h].astype(BF16), v[h].astype(BF16))

            def do_wo(h, acc):
                r = _dot(o[h].astype(BF16), wob[h * E:(h + 1) * E, :])
                return r if acc is None else acc + r

            for t in range(HB):
                do_qkv(t)
                if t >= ls:
                    do_s(t - ls)
                if t >= lp:
                    do_pv(t - lp)
                for f in hooks.get(t, ()):
                    f()
            acc = None
            wo_next = 0
            for t in range(HB, HB + lp):
                for _ in range(nfill):
                    if wo_next < t - lp:
                        acc = do_wo(wo_next, acc)
                        wo_next += 1
                if t - ls < HB:
                    do_s(t - ls)
                do_pv(t - lp)
            for h in range(wo_next, HB):
                acc = do_wo(h, acc)
            for f in hooks.get("end", ()):
                f()
            return acc, kv

        def pair(base, mem, hooksE, hooksO):
            t8 = xb[pl.ds(base, 8), :].astype(F32)
            g0 = jnp.concatenate([mem, t8], axis=0).astype(BF16)
            g12 = xb[pl.ds(base + 8, 32), :]
            hA = jnp.concatenate([g0, g12], axis=0)
            resA, kvA = seg_step(hA[0:32], hA, None, capE, hooksE, *LAG_E)
            mem1 = resA[0:8].astype(BF16).astype(F32)
            t8b = xb[pl.ds(base + 40, 8), :].astype(F32)
            g0b = jnp.concatenate([mem1, t8b], axis=0).astype(BF16)
            g1b = xb[pl.ds(base + 48, 16), :]
            hB = jnp.concatenate([g0b, g1b], axis=0)
            hQ = jnp.concatenate([hB, hA[32:48]], axis=0)
            resB, _ = seg_step(hQ, hB, kvA, capO, hooksO, *LAG_O)
            mem2 = resB[0:8].astype(BF16).astype(F32)
            b64 = jnp.concatenate([resA[8:32], resB[32:48], resB[8:32]], axis=0)
            bb[pl.ds(base, 64), :] = b64.astype(BF16)
            return mem2

        def combine(c0):
            bT = bb[pl.ds(c0, QB), :].T.astype(F32)
            g = gl[0:1, pl.ds(c0, QB)]
            outT[:, pl.ds(c0, QB)] = (gaT[:, pl.ds(c0, QB)] + (1.0 - g) * bT).astype(BF16)

        def out_copy(b):
            c0 = pl.multiple_of(b * QB, QB)
            return pltpu.make_async_copy(outT.at[:, pl.ds(c0, QB)], outT_hbm.at[:, pl.ds(c0, QB)], sems.at[16 + b])

        def super_iter(j, mem):
            q0 = pl.multiple_of(j * QB, QB)
            sc = {}
            oTs = [None] * HA

            def keep_scores(g, r):
                for jj in range(GPH):
                    sc[g * GPH + jj] = r[:, jj * QB:(jj + 1) * QB]

            def finish(h):
                oTs[h] = a_finish(q0, h, sc[h])

            def next_scores():
                qn = pl.multiple_of(jnp.minimum(j + 1, NQB - 1) * QB, QB)
                s0buf[...] = a_scores(qn, 0)

            hk = []
            for g in range(NG):
                h_g = {}
                for jj in range(GPH):
                    h_g.setdefault(FIN_T[jj], []).append(functools.partial(finish, g * GPH + jj))
                if g + 1 < NG:
                    h_g["end"] = [lambda g=g: keep_scores(g + 1, a_scores(q0, g + 1))]
                else:
                    h_g.setdefault(AOUT_T, []).append(lambda: a_out(q0, oTs))
                    h_g["end"] = [next_scores]
                hk.append(h_g)
            hk[0].setdefault(COMB_T, []).append(
                lambda: combine(pl.multiple_of(jnp.maximum(j - 1, 0) * QB, QB)))

            keep_scores(0, s0buf[...])
            mem = pair(q0, mem, hk[0], hk[1])
            mem = pair(q0 + 64, mem, hk[2], hk[3])
            return mem

        def double_iter(i, mem):
            mem = super_iter(2 * i, mem)
            mem = super_iter(2 * i + 1, mem)
            out_copy(2 * i).start()

            @pl.when(i > 0)
            def _():
                out_copy(2 * i - 1).start()
            return mem

        s0buf[...] = a_scores(0, 0)
        lax.fori_loop(0, NQB // 2, double_iter, mem0_ref[...].astype(F32))
        combine((NQB - 1) * QB)
        out_copy(NQB - 1).start()
        for b in range(NQB):
            out_copy(b).wait()

    return kernel


@functools.partial(jax.jit, static_argnames=("B_seg_len",))
def pallas_gated_mix__sliding_block__memory_aug_recurrent_mem_tr__prompt_kernel(
        A_x, A_wqkv, A_wo, B_x, B_mem0, B_Wq, B_Wk, B_Wv, B_Wo, B_seg_len, gate_w):
    del B_x
    Bn, S, D = A_x.shape
    assert Bn == 1
    HB, E = B_Wq.shape[1], B_Wq.shape[2]
    M = B_mem0.shape[1]
    HA, WIN = 16, 256
    kern = _make_kernel(S, D, HA, WIN, HB, E, M, B_seg_len)
    hbm_spec = pl.BlockSpec(memory_space=pltpu.MemorySpace.HBM)
    outT = pl.pallas_call(
        kern,
        out_shape=jax.ShapeDtypeStruct((D, S), BF16),
        in_specs=[hbm_spec] * 9,
        out_specs=hbm_spec,
        scratch_shapes=[
            pltpu.VMEM((D, S), BF16),
            pltpu.VMEM((D, 3 * D), BF16),
            pltpu.VMEM((D, D), BF16),
            pltpu.VMEM((S, D), BF16),
            pltpu.VMEM((4, D * HB // 4 + 8, 128), U32),
            pltpu.VMEM((4, D * HB // 2 + 16, 128), U32),
            pltpu.VMEM((D // 2, 3 * HB * E), U32),
            pltpu.VMEM((HB * D, E), BF16),
            pltpu.VMEM((HB * E, D), BF16),
            pltpu.VMEM((3 * D + 16, D), BF16),
            pltpu.VMEM((D, 512), BF16),
            pltpu.VMEM((512, S), BF16),
            pltpu.VMEM((WIN + S, 512), BF16),
            pltpu.VMEM((512, WIN + S), BF16),
            pltpu.VMEM((8, S), F32),
            pltpu.VMEM((D, S), F32),
            pltpu.VMEM((S, D), BF16),
            pltpu.VMEM((D, S), BF16),
            pltpu.VMEM((3 * 128, 512), F32),
            pltpu.VMEM((M, D), BF16),
            pltpu.VMEM((D,), BF16),
            pltpu.SemaphoreType.DMA((46,)),
        ],
        compiler_params=pltpu.CompilerParams(vmem_limit_bytes=110 * 1024 * 1024),
    )(A_x.reshape(S, D).T, A_wqkv, A_wo, B_mem0.reshape(M, D),
      B_Wq.reshape(D // 2, 2 * HB, E), B_Wk.reshape(D // 2, 2 * HB, E), B_Wv.reshape(D // 2, 2 * HB, E),
      jnp.transpose(B_Wo, (0, 2, 1)).reshape(HB * D, E), gate_w)
    return outT.T.reshape(1, S, D)
```
